```python
import jax
import jax.numpy as jnp

def _softmax(x, axis=-1):
    return jax.nn.softmax(x, axis=axis)
def _gelu(x):
    return jax.nn.gelu(x, approximate=True)
def _silu(x):
    return jax.nn.silu(x)
def _sigmoid(x):
    return jax.nn.sigmoid(x)
def _layernorm(x, axis=-1, eps=1e-5):
    m = jnp.mean(x, axis=axis, keepdims=True)
    v = jnp.var(x, axis=axis, keepdims=True)
    return (x - m) / jnp.sqrt(v + eps)
def _scatter_add(tgt, idx, src, axis=0):
    return tgt.at[idx].add(src)
def _segment_sum(src, seg, n):
    return jax.ops.segment_sum(src, seg, n)
class _Rng:
    def __init__(self, key):
        self._k = key
    def _next(self):
        self._k, sub = jax.random.split(self._k)
        return sub
    def normal(self, shape):
        return jax.random.normal(self._next(), shape, dtype=jnp.bfloat16)
    def randint(self, lo, hi, shape):
        return jax.random.randint(self._next(), shape, lo, hi, dtype=jnp.int32)
    def uniform(self, shape, lo=0.0, hi=1.0):
        return jax.random.uniform(self._next(), shape, jnp.bfloat16, lo, hi)
    def permutation(self, n):
        return jax.random.permutation(self._next(), n)


kernel_name = 'interleave_layers__sliding_block_cached__moe_arch_mod__decode'

def setup_inputs():
    _rng = _Rng(jax.random.key(int.from_bytes(__import__("os").urandom(4), "little")))
    _w = (lambda a: (lambda t: t.astype(jnp.bfloat16) if jnp.issubdtype(t.dtype, jnp.floating) else t)(jnp.asarray(a)))
    def _A_setup():
        B, Sq, D = 4, 1, 640
        Hq, Hkv, Sk, Dh = 32, 32, 4096, 192
        assert Hq % Hkv == 0, (Hq, Hkv)
        return {
            "x": _w((lambda *s: _rng.normal(s) * 0.05)(B, Sq, D)),
            "k_cache": _w((lambda *s: _rng.normal(s) * 0.05)(B, Hkv, Sk, Dh)),
            "v_cache": _w((lambda *s: _rng.normal(s) * 0.05)(B, Hkv, Sk, Dh)),
            "wq": _w((lambda *s: _rng.normal(s) * 0.05)(D, Hq * Dh) * (D ** -0.5)),
            "wo": _w((lambda *s: _rng.normal(s) * 0.05)(Hq * Dh, D) * ((Hq * Dh) ** -0.5)),
        }
    _A_in = _A_setup()

    def _B_setup():
        B, S, D, F, C = 4, 1, 640, 1536, 1
        return {
            "x": _w((lambda *s: _rng.normal(s) * 0.05)(B, S, D)),
            "w_r": _w((lambda *s: _rng.normal(s) * 0.05)(D)),
            "w_gate": _w((lambda *s: _rng.normal(s) * 0.05)(D, F)),
            "w_up": _w((lambda *s: _rng.normal(s) * 0.05)(D, F)),
            "w_down": _w((lambda *s: _rng.normal(s) * 0.05)(F, D)),
        }
    _B_in = _B_setup()

    return {
        "A_x": _A_in["x"],
        "A_k_cache": _A_in["k_cache"],
        "A_v_cache": _A_in["v_cache"],
        "A_wq": _A_in["wq"],
        "A_wo": _A_in["wo"],
        "B_x": _B_in["x"],
        "B_w_r": _B_in["w_r"],
        "B_w_gate": _B_in["w_gate"],
        "B_w_up": _B_in["w_up"],
        "B_w_down": _B_in["w_down"],
    }

def reference(A_x, A_k_cache, A_v_cache, A_wq, A_wo, B_x, B_w_r, B_w_gate, B_w_up, B_w_down):
    def _A_ref(x, k_cache, v_cache, wq, wo):
        B, Sq, D = x.shape
        Hq, Dh = 32, 192
        Hkv, Sk = k_cache.shape[1], k_cache.shape[2]
        W = min(4096, max(256, Sk // 4))
        rep = Hq // Hkv
        q = (lambda x, *d: x.transpose(*d))((x @ wq).reshape(B, Sq, Hq, Dh), 0, 2, 1, 3)
        k = jnp.repeat(k_cache[:, :, Sk - W:, :], rep, axis=1)
        v = jnp.repeat(v_cache[:, :, Sk - W:, :], rep, axis=1)
        scores = jnp.einsum("bhqd,bhkd->bhqk", q, k) * (Dh ** -0.5)
        p = _softmax(scores, axis=-1)
        o = jnp.einsum("bhqk,bhkd->bhqd", p, v)
        return (lambda x, *d: x.transpose(*d))(o, 0, 2, 1, 3).reshape(B, Sq, Hq * Dh) @ wo

    def _B_ref(x, w_r, w_gate, w_up, w_down):
        B, S, D = x.shape
        C = 1
        r = x @ w_r
        idx = jnp.argsort(-r, axis=-1)[:, :C]
        idx_e = jnp.repeat(idx.reshape(B, C, 1), D, axis=2)
        x_sel = jnp.take_along_axis(x, idx_e, axis=1)
        g = _silu(x_sel @ w_gate)
        u = x_sel @ w_up
        y = (g * u) @ w_down
        r_sel = _sigmoid(jnp.take_along_axis(r, idx, axis=1))
        y = y * r_sel.reshape(B, C, 1)
        b_off = (jnp.arange(B) * S).reshape(B, 1)
        flat_idx = (idx + b_off).reshape(B * C)
        zero = (x * 0.0).reshape(B * S, D)
        upd = _scatter_add(zero, flat_idx, y.reshape(B * C, D), axis=0)
        return x + upd.reshape(B, S, D)

    x = A_x
    x = x + _A_ref(_layernorm(x, axis=-1), A_k_cache, A_v_cache, A_wq, A_wo)
    x = x + _B_ref(_layernorm(x, axis=-1), B_w_r, B_w_gate, B_w_up, B_w_down)
    x = x + _A_ref(_layernorm(x, axis=-1), A_k_cache, A_v_cache, A_wq, A_wo)
    x = x + _B_ref(_layernorm(x, axis=-1), B_w_r, B_w_gate, B_w_up, B_w_down)
    return x
```

```python
import jax
import jax.numpy as jnp
from jax import lax
import jax.experimental.pallas as pl
import jax.experimental.pallas.tpu as pltpu

F32 = jnp.float32
BF16 = jnp.bfloat16

_HQ = 32
_DH = 192
_G = 8
_NB = 2


def _layernorm(x, eps=1e-5):
    m = jnp.mean(x, axis=-1, keepdims=True)
    xc = x - m
    v = jnp.mean(xc * xc, axis=-1, keepdims=True)
    return xc * lax.rsqrt(v + eps)


@jax.jit
def pallas_interleave_layers__sliding_block_cached__moe_arch_mod__decode_kernel(
    A_x: jax.Array,
    A_k_cache: jax.Array,
    A_v_cache: jax.Array,
    A_wq: jax.Array,
    A_wo: jax.Array,
    B_x: jax.Array,
    B_w_r: jax.Array,
    B_w_gate: jax.Array,
    B_w_up: jax.Array,
    B_w_down: jax.Array,
):
    del B_x
    B, Sq, D = A_x.shape
    _, Hkv, Sk, Dh = A_k_cache.shape
    assert Sq == 1 and Hkv == _HQ and Dh == _DH
    F = B_w_gate.shape[1]
    W = min(4096, max(256, Sk // 4))
    HD = _HQ * _DH
    G = _G
    NG = _HQ // G
    GD = G * _DH
    NB = _NB
    WH = W // 2
    scale = float(_DH) ** -0.5

    def kernel(x_ref, wr_ref, k_hbm, v_hbm, wq_hbm, wo_hbm, wg_hbm, wu_hbm, wd_hbm,
               out_ref,
               kbuf, vbuf, wq, wo, wg, wu, wd, x_scr, s_scr, p_scr, l_scr,
               ksem, vsem, wsem):

        def k_copy(b, g, half):
            slot = b % NB
            return pltpu.make_async_copy(
                k_hbm.at[b, pl.ds(g * GD, GD), pl.ds(Sk - W + half * WH, WH)],
                kbuf.at[slot, g, half], ksem.at[slot, g, half])

        def v_copy(b, g):
            slot = b % NB
            return pltpu.make_async_copy(
                v_hbm.at[b, pl.ds(g * GD, GD), pl.ds(Sk - W, W)],
                vbuf.at[slot, g], vsem.at[slot, g])

        def wq_copy(g):
            return pltpu.make_async_copy(
                wq_hbm.at[:, pl.ds(g * GD, GD)], wq.at[g], wsem.at[g])

        def wo_copy(g):
            return pltpu.make_async_copy(
                wo_hbm.at[pl.ds(g * GD, GD), :], wo.at[g], wsem.at[NG + g])

        ffn_copies = [
            pltpu.make_async_copy(wg_hbm, wg, wsem.at[2 * NG]),
            pltpu.make_async_copy(wu_hbm, wu, wsem.at[2 * NG + 1]),
            pltpu.make_async_copy(wd_hbm, wd, wsem.at[2 * NG + 2]),
        ]

        def start_kv(b):
            for g in range(NG):
                k_copy(b, g, 0).start()
                k_copy(b, g, 1).start()
            for g in range(NG):
                v_copy(b, g).start()

        for g in range(NG):
            wq_copy(g).start()
            k_copy(0, g, 0).start()
            k_copy(0, g, 1).start()
        for g in range(NG):
            v_copy(0, g).start()
            wo_copy(g).start()
        for c in ffn_copies:
            c.start()
        for b in range(1, NB):
            start_kv(b)

        x_in = x_ref[...].astype(F32)
        for b in range(B):
            x_scr[b] = jnp.broadcast_to(x_in[b:b + 1, :], (8, D))
        w_r = wr_ref[...].astype(F32).reshape(1, D)

        row = lax.broadcasted_iota(jnp.int32, (G, GD), 0)
        col = lax.broadcasted_iota(jnp.int32, (G, GD), 1)
        diag = (col >= row * _DH) & (col < (row + 1) * _DH)

        def step(i, carry):
            b = i // 2
            first = (i % 2) == 0
            slot = b % NB
            x = x_scr[b]

            xn = _layernorm(x).astype(BF16)

            def qk_group(g, c):
                @pl.when(i == 0)
                def _():
                    wq_copy(g).wait()

                q = jnp.dot(xn, wq[g], preferred_element_type=F32)
                qbd = jnp.where(diag, q, 0.0).astype(BF16)

                @pl.when(first)
                def _():
                    k_copy(b, g, 0).wait()
                    k_copy(b, g, 1).wait()

                for half in range(2):
                    s_scr[g, :, pl.ds(half * WH, WH)] = jnp.dot(
                        qbd, kbuf[slot, g, half], preferred_element_type=F32)
                return c

            lax.fori_loop(0, NG, qk_group, 0)

            s = s_scr[...].reshape(NG * G, W) * scale
            m = jnp.max(s, axis=-1, keepdims=True)
            p = jnp.exp(s - m)
            l = jnp.sum(p, axis=-1, keepdims=True)
            p_scr[...] = p.reshape(NG, G, W)
            l_scr[...] = jnp.broadcast_to(1.0 / l, (NG * G, 128)).reshape(NG, G, 128)

            def pv_group(g, acc):
                @pl.when(first)
                def _():
                    v_copy(b, g).wait()

                pg = p_scr[g].astype(BF16)
                o = lax.dot_general(pg, vbuf[slot, g], (((1,), (1,)), ((), ())),
                                    preferred_element_type=F32)
                o = jnp.where(diag, o * l_scr[g][:, 0:1], 0.0).astype(BF16)

                @pl.when(i == 0)
                def _():
                    wo_copy(g).wait()

                return acc + jnp.dot(o, wo[g], preferred_element_type=F32)

            acc = lax.fori_loop(0, NG, pv_group, jnp.zeros((8, D), F32))

            @pl.when(jnp.logical_and(jnp.logical_not(first), b + NB < B))
            def _():
                start_kv(b + NB)

            x = x + jnp.sum(acc, axis=0, keepdims=True)

            @pl.when(i == 0)
            def _():
                ffn_copies[0].wait()
                ffn_copies[1].wait()
                ffn_copies[2].wait()

            xn32 = _layernorm(x)
            xnb = xn32.astype(BF16)
            xnr = xnb.astype(F32)
            r = jnp.sum(xnr * w_r, axis=-1, keepdims=True)
            gate = jnp.dot(xnb, wg[...], preferred_element_type=F32)
            up = jnp.dot(xnb, wu[...], preferred_element_type=F32)
            h = (gate * jax.nn.sigmoid(gate) * up).astype(BF16)
            y = jnp.dot(h, wd[...], preferred_element_type=F32)
            x_scr[b] = x + (xnr + y * jax.nn.sigmoid(r))
            return carry

        lax.fori_loop(0, 2 * B, step, 0)

        out = jnp.concatenate([x_scr[b][0:1, :] for b in range(B)], axis=0)
        out_ref[...] = out.astype(out_ref.dtype)

    kt = jnp.transpose(A_k_cache, (0, 1, 3, 2)).reshape(B, HD, Sk)
    vt = jnp.transpose(A_v_cache, (0, 1, 3, 2)).reshape(B, HD, Sk)
    x2 = A_x.reshape(B, D)

    hbm = pl.BlockSpec(memory_space=pltpu.HBM)
    vmem = pl.BlockSpec(memory_space=pltpu.VMEM)
    out = pl.pallas_call(
        kernel,
        out_shape=jax.ShapeDtypeStruct((B, D), A_x.dtype),
        in_specs=[vmem, vmem] + [hbm] * 7,
        out_specs=vmem,
        scratch_shapes=[
            pltpu.VMEM((NB, NG, 2, GD, WH), BF16),
            pltpu.VMEM((NB, NG, GD, W), BF16),
            pltpu.VMEM((NG, D, GD), BF16),
            pltpu.VMEM((NG, GD, D), BF16),
            pltpu.VMEM((D, F), BF16),
            pltpu.VMEM((D, F), BF16),
            pltpu.VMEM((F, D), BF16),
            pltpu.VMEM((B, 8, D), F32),
            pltpu.VMEM((NG, G, W), F32),
            pltpu.VMEM((NG, G, W), F32),
            pltpu.VMEM((NG, G, 128), F32),
            pltpu.SemaphoreType.DMA((NB, NG, 2)),
            pltpu.SemaphoreType.DMA((NB, NG)),
            pltpu.SemaphoreType.DMA((2 * NG + 3,)),
        ],
        compiler_params=pltpu.CompilerParams(vmem_limit_bytes=100 * 1024 * 1024),
    )(x2, B_w_r, kt, vt, A_wq, A_wo, B_w_gate, B_w_up, B_w_down)
    return out.reshape(B, Sq, D)
```

```python
import jax
import jax.numpy as jnp
from jax import lax
import jax.experimental.pallas as pl
import jax.experimental.pallas.tpu as pltpu

F32 = jnp.float32
BF16 = jnp.bfloat16

_HQ = 32
_DH = 192
_G = 8
_NB = 4


def _layernorm(x, eps=1e-5):
    m = jnp.mean(x, axis=-1, keepdims=True)
    xc = x - m
    v = jnp.mean(xc * xc, axis=-1, keepdims=True)
    return xc * lax.rsqrt(v + eps)


@jax.jit
def pallas_interleave_layers__sliding_block_cached__moe_arch_mod__decode_kernel(
    A_x: jax.Array,
    A_k_cache: jax.Array,
    A_v_cache: jax.Array,
    A_wq: jax.Array,
    A_wo: jax.Array,
    B_x: jax.Array,
    B_w_r: jax.Array,
    B_w_gate: jax.Array,
    B_w_up: jax.Array,
    B_w_down: jax.Array,
):
    del B_x
    B, Sq, D = A_x.shape
    _, Hkv, Sk, Dh = A_k_cache.shape
    assert Sq == 1 and Hkv == _HQ and Dh == _DH
    F = B_w_gate.shape[1]
    W = min(4096, max(256, Sk // 4))
    HD = _HQ * _DH
    G = _G
    NG = _HQ // G
    GD = G * _DH
    NB = _NB
    WH = W // 2
    NKV = NB * NG * 3
    scale = float(_DH) ** -0.5

    def kernel(x_ref, wr_ref, k_hbm, v_hbm, wq_hbm, wo_hbm, wg_hbm, wu_hbm, wd_hbm,
               out_ref,
               kbuf, vbuf, wq, wo, wg, wu, wd, x_scr, s_scr, p_scr, l_scr,
               sems):

        def k_copy(b, g, half):
            slot = b % NB
            return pltpu.make_async_copy(
                k_hbm.at[b, pl.ds(g * GD, GD), pl.ds(Sk - W + half * WH, WH)],
                kbuf.at[slot, g, half], sems.at[(slot * NG + g) * 3 + half])

        def v_copy(b, g):
            slot = b % NB
            return pltpu.make_async_copy(
                v_hbm.at[b, pl.ds(g * GD, GD), pl.ds(Sk - W, W)],
                vbuf.at[slot, g], sems.at[(slot * NG + g) * 3 + 2])

        def wq_copy(g):
            return pltpu.make_async_copy(
                wq_hbm.at[:, pl.ds(g * GD, GD)], wq.at[g], sems.at[NKV + g])

        def wo_copy(g):
            return pltpu.make_async_copy(
                wo_hbm.at[pl.ds(g * GD, GD), :], wo.at[g], sems.at[NKV + NG + g])

        ffn_copies = [
            pltpu.make_async_copy(wg_hbm, wg, sems.at[NKV + 2 * NG]),
            pltpu.make_async_copy(wu_hbm, wu, sems.at[NKV + 2 * NG + 1]),
            pltpu.make_async_copy(wd_hbm, wd, sems.at[NKV + 2 * NG + 2]),
        ]

        def start_kv(b):
            for g in range(NG):
                k_copy(b, g, 0).start()
                k_copy(b, g, 1).start()
            for g in range(NG):
                v_copy(b, g).start()

        for g in range(NG):
            wq_copy(g).start()
            k_copy(0, g, 0).start()
            k_copy(0, g, 1).start()
        for g in range(NG):
            v_copy(0, g).start()
            wo_copy(g).start()
        for c in ffn_copies:
            c.start()
        for b in range(1, NB):
            start_kv(b)

        x_in = x_ref[...].astype(F32)
        for b in range(B):
            x_scr[b] = jnp.broadcast_to(x_in[b:b + 1, :], (8, D))
        w_r = wr_ref[...].astype(F32).reshape(1, D)

        row = lax.broadcasted_iota(jnp.int32, (G, GD), 0)
        col = lax.broadcasted_iota(jnp.int32, (G, GD), 1)
        diag = (col >= row * _DH) & (col < (row + 1) * _DH)

        def step(i, carry):
            b = i // 2
            first = (i % 2) == 0
            slot = b % NB
            x = x_scr[b]

            xn = _layernorm(x).astype(BF16)

            def qk_group(g, c):
                @pl.when(i == 0)
                def _():
                    wq_copy(g).wait()

                q = jnp.dot(xn, wq[g], preferred_element_type=F32)
                qbd = jnp.where(diag, q, 0.0).astype(BF16)

                @pl.when(first)
                def _():
                    k_copy(b, g, 0).wait()
                    k_copy(b, g, 1).wait()

                for half in range(2):
                    s_scr[g, :, pl.ds(half * WH, WH)] = jnp.dot(
                        qbd, kbuf[slot, g, half], preferred_element_type=F32)
                return c

            lax.fori_loop(0, NG, qk_group, 0)

            s = s_scr[...].reshape(NG * G, W) * scale
            m = jnp.max(s, axis=-1, keepdims=True)
            p = jnp.exp(s - m)
            l = jnp.sum(p, axis=-1, keepdims=True)
            p_scr[...] = p.reshape(NG, G, W)
            l_scr[...] = jnp.broadcast_to(1.0 / l, (NG * G, 128)).reshape(NG, G, 128)

            def pv_group(g, acc):
                @pl.when(first)
                def _():
                    v_copy(b, g).wait()

                pg = p_scr[g].astype(BF16)
                o = lax.dot_general(pg, vbuf[slot, g], (((1,), (1,)), ((), ())),
                                    preferred_element_type=F32)
                o = jnp.where(diag, o * l_scr[g][:, 0:1], 0.0).astype(BF16)

                @pl.when(i == 0)
                def _():
                    wo_copy(g).wait()

                return acc + jnp.dot(o, wo[g], preferred_element_type=F32)

            acc = lax.fori_loop(0, NG, pv_group, jnp.zeros((8, D), F32))

            if NB < B:
                @pl.when(jnp.logical_and(jnp.logical_not(first), b + NB < B))
                def _():
                    start_kv(b + NB)

            x = x + jnp.sum(acc, axis=0, keepdims=True)

            @pl.when(i == 0)
            def _():
                ffn_copies[0].wait()
                ffn_copies[1].wait()
                ffn_copies[2].wait()

            xn32 = _layernorm(x)
            xnb = xn32.astype(BF16)
            xnr = xnb.astype(F32)
            r = jnp.sum(xnr * w_r, axis=-1, keepdims=True)
            gate = jnp.dot(xnb, wg[...], preferred_element_type=F32)
            up = jnp.dot(xnb, wu[...], preferred_element_type=F32)
            h = (gate * jax.nn.sigmoid(gate) * up).astype(BF16)
            y = jnp.dot(h, wd[...], preferred_element_type=F32)
            x_scr[b] = x + (xnr + y * jax.nn.sigmoid(r))
            return carry

        lax.fori_loop(0, 2 * B, step, 0)

        out = jnp.concatenate([x_scr[b][0:1, :] for b in range(B)], axis=0)
        out_ref[...] = out.astype(out_ref.dtype)

    kt = jnp.transpose(A_k_cache, (0, 1, 3, 2)).reshape(B, HD, Sk)
    vt = jnp.transpose(A_v_cache, (0, 1, 3, 2)).reshape(B, HD, Sk)
    x2 = A_x.reshape(B, D)

    hbm = pl.BlockSpec(memory_space=pltpu.HBM)
    vmem = pl.BlockSpec(memory_space=pltpu.VMEM)
    out = pl.pallas_call(
        kernel,
        out_shape=jax.ShapeDtypeStruct((B, D), A_x.dtype),
        in_specs=[vmem, vmem] + [hbm] * 7,
        out_specs=vmem,
        scratch_shapes=[
            pltpu.VMEM((NB, NG, 2, GD, WH), BF16),
            pltpu.VMEM((NB, NG, GD, W), BF16),
            pltpu.VMEM((NG, D, GD), BF16),
            pltpu.VMEM((NG, GD, D), BF16),
            pltpu.VMEM((D, F), BF16),
            pltpu.VMEM((D, F), BF16),
            pltpu.VMEM((F, D), BF16),
            pltpu.VMEM((B, 8, D), F32),
            pltpu.VMEM((NG, G, W), F32),
            pltpu.VMEM((NG, G, W), F32),
            pltpu.VMEM((NG, G, 128), F32),
            pltpu.SemaphoreType.DMA((NKV + 2 * NG + 3,)),
        ],
        compiler_params=pltpu.CompilerParams(vmem_limit_bytes=127 * 1024 * 1024),
    )(x2, B_w_r, kt, vt, A_wq, A_wo, B_w_gate, B_w_up, B_w_down)
    return out.reshape(B, Sq, D)
```

```python
import jax
import jax.numpy as jnp
from jax import lax
import jax.experimental.pallas as pl
import jax.experimental.pallas.tpu as pltpu

F32 = jnp.float32
BF16 = jnp.bfloat16
_HQ, _DH = 32, 192


def _layernorm(x, eps=1e-5):
    m = jnp.mean(x, axis=-1, keepdims=True)
    xc = x - m
    v = jnp.mean(xc * xc, axis=-1, keepdims=True)
    return xc * lax.rsqrt(v + eps)


@jax.jit
def pallas_interleave_layers__sliding_block_cached__moe_arch_mod__decode_kernel(
    A_x, A_k_cache, A_v_cache, A_wq, A_wo, B_x, B_w_r, B_w_gate, B_w_up, B_w_down):
    del B_x
    B, Sq, D = A_x.shape
    _, Hkv, Sk, Dh = A_k_cache.shape
    F = B_w_gate.shape[1]
    W = min(4096, max(256, Sk // 4))
    HD = _HQ * _DH
    G = 8
    NG = _HQ // G
    GD = G * _DH
    NU = 2 * NG
    UD = HD // NU
    UH = UD // _DH
    WH = W // 2
    NJ = W // 128
    scale = float(_DH) ** -0.5
    NT = (((1,), (1,)), ((), ()))

    def kernel(x_hbm, wr_hbm, k_hbm, v_hbm, wq_hbm, wo_hbm, wg_hbm, wu_hbm, wd_hbm,
               out_ref,
               xin, wr, kbuf, vbuf, wq, wo, wg, wu, wd, x_scr, q_scr, s_scr, p_scr, o_scr, sems):
        KS = 0
        VS = B * NG * 2
        WS = VS + B * NU

        def k_copy(b, g, half):
            return pltpu.make_async_copy(
                k_hbm.at[b, pl.ds(g * GD, GD), pl.ds(Sk - W + half * WH, WH)],
                kbuf.at[b, g, half], sems.at[KS + b * NG * 2 + g * 2 + half])

        def v_copy(b, u):
            return pltpu.make_async_copy(
                v_hbm.at[b, pl.ds(u * UD, UD), pl.ds(Sk - W, W)],
                vbuf.at[b, u], sems.at[VS + b * NU + u])

        def wq_copy(g):
            return pltpu.make_async_copy(wq_hbm.at[:, pl.ds(g * GD, GD)], wq.at[g], sems.at[WS + g])

        def wo_copy(g):
            return pltpu.make_async_copy(wo_hbm.at[pl.ds(g * GD, GD), :], wo.at[pl.ds(g * GD, GD), :], sems.at[WS + NG + g])

        small = [
            pltpu.make_async_copy(wg_hbm, wg, sems.at[WS + 2 * NG]),
            pltpu.make_async_copy(wu_hbm, wu, sems.at[WS + 2 * NG + 1]),
            pltpu.make_async_copy(wd_hbm, wd, sems.at[WS + 2 * NG + 2]),
            pltpu.make_async_copy(x_hbm, xin, sems.at[WS + 2 * NG + 3]),
            pltpu.make_async_copy(wr_hbm, wr, sems.at[WS + 2 * NG + 4]),
        ]

        small[3].start()
        small[4].start()
        for g in range(NG):
            wq_copy(g).start()
        for g in range(NG):
            k_copy(0, g, 0).start()
            k_copy(0, g, 1).start()
        for u in range(NU):
            v_copy(0, u).start()
            if u % 2 == 1:
                wo_copy(u // 2).start()
        for c in small[:3]:
            c.start()
        for b in range(1, B):
            for g in range(NG):
                k_copy(b, g, 0).start()
                k_copy(b, g, 1).start()
            for u in range(NU):
                v_copy(b, u).start()

        small[3].wait()
        small[4].wait()
        x_in = xin[...].astype(F32)
        for b in range(B):
            x_scr[b] = jnp.broadcast_to(x_in[b:b + 1, :], (8, D))
        w_r = wr[...].astype(F32).reshape(1, D)

        row = lax.broadcasted_iota(jnp.int32, (G, GD), 0)
        col = lax.broadcasted_iota(jnp.int32, (G, GD), 1)
        diag = (col >= row * _DH) & (col < (row + 1) * _DH)
        diag_u = [diag[:, :UD], diag[:, UD:]]

        def transpose_unit(b, u):
            for n in range(UD // 128):
                for j in range(NJ):
                    sl = (b, u, pl.ds(n * 128, 128), pl.ds(j * 128, 128))
                    vbuf[sl] = vbuf[sl].T

        def pv_xpose(b, u, pg):
            return lax.dot_general(pg, vbuf[b, u], NT, preferred_element_type=F32)

        def pv_plain(b, u, pg):
            outs = []
            for n in range(UD // 128):
                acc = None
                for j in range(NJ):
                    d = jnp.dot(pg[:, j * 128:(j + 1) * 128],
                                vbuf[b, u, pl.ds(n * 128, 128), pl.ds(j * 128, 128)],
                                preferred_element_type=F32)
                    acc = d if acc is None else acc + d
                outs.append(acc)
            return jnp.concatenate(outs, axis=1)

        def step(i, carry):
            b = i // 2
            first = (i % 2) == 0
            x = x_scr[b]
            xn = _layernorm(x).astype(BF16)

            def q_group(g, c):
                @pl.when(i == 0)
                def _():
                    wq_copy(g).wait()
                q_scr[g] = jnp.dot(xn, wq[g], preferred_element_type=F32)
                return c
            lax.fori_loop(0, NG, q_group, 0)

            def qk_group(g, c):
                qbd = jnp.where(diag, q_scr[g], 0.0).astype(BF16)

                @pl.when(first)
                def _():
                    k_copy(b, g, 0).wait()
                    k_copy(b, g, 1).wait()

                for half in range(2):
                    s_scr[g, :, pl.ds(half * WH, WH)] = jnp.dot(
                        qbd, kbuf[b, g, half], preferred_element_type=F32)
                return c
            lax.fori_loop(0, NG, qk_group, 0)

            s = s_scr[...].reshape(NG * G, W) * scale
            m = jnp.max(s, axis=-1, keepdims=True)
            p = jnp.exp(s - m)
            l = jnp.sum(p, axis=-1, keepdims=True)
            p_scr[...] = (p / l).reshape(NG, G, W)

            def finish(o, u):
                return jnp.where(diag_u[u % 2], o, 0.0).astype(BF16)

            @pl.when(first)
            def _():
                def unit(u2, acc):
                    for r in range(2):
                        u = u2 * 2 + r

                        @pl.when(u > 0)
                        def _():
                            transpose_unit(b, u - 1)
                        v_copy(b, u).wait()
                        pg = p_scr[u2].astype(BF16)
                        o = finish(pv_xpose(b, u, pg), r)
                        if r == 0:
                            @pl.when(i == 0)
                            def _():
                                wo_copy(u2).wait()
                        acc = acc + jnp.dot(o, wo[pl.ds(pl.multiple_of(u * UD, UD), UD), :], preferred_element_type=F32)
                    return acc
                acc = lax.fori_loop(0, NG, unit, jnp.zeros((8, D), F32))
                o_scr[...] = acc

            @pl.when(jnp.logical_not(first))
            def _():
                acc = jnp.zeros((8, D), F32)
                os_ = []
                for u in range(NU):
                    pg = p_scr[u // 2].astype(BF16)
                    o = pv_plain(b, u, pg) if u < NU - 1 else pv_xpose(b, u, pg)
                    os_.append(finish(o, u))
                ocat = jnp.concatenate(os_, axis=1)
                o_scr[...] = jnp.dot(ocat, wo[...], preferred_element_type=F32)

            @pl.when(i == 0)
            def _():
                small[0].wait()
                small[1].wait()
                small[2].wait()
            x = x + jnp.sum(o_scr[...], axis=0, keepdims=True)
            xnb = _layernorm(x).astype(BF16)
            xnr = xnb.astype(F32)
            r = jnp.sum(xnr * w_r, axis=-1, keepdims=True)
            gate = jnp.dot(xnb, wg[...], preferred_element_type=F32)
            up = jnp.dot(xnb, wu[...], preferred_element_type=F32)
            h = (gate * jax.nn.sigmoid(gate) * up).astype(BF16)
            y = jnp.dot(h, wd[...], preferred_element_type=F32)
            x_scr[b] = x + (xnr + y * jax.nn.sigmoid(r))
            return carry

        lax.fori_loop(0, 2 * B, step, 0)

        out = jnp.concatenate([x_scr[b][0:1, :] for b in range(B)], axis=0)
        out_ref[...] = out.astype(out_ref.dtype)

    kt = jnp.transpose(A_k_cache, (0, 1, 3, 2)).reshape(B, HD, Sk)
    vt = jnp.transpose(A_v_cache, (0, 1, 3, 2)).reshape(B, HD, Sk)
    x2 = A_x.reshape(B, D)

    hbm = pl.BlockSpec(memory_space=pltpu.HBM)
    vmem = pl.BlockSpec(memory_space=pltpu.VMEM)
    out = pl.pallas_call(
        kernel,
        out_shape=jax.ShapeDtypeStruct((B, D), A_x.dtype),
        in_specs=[hbm] * 9,
        out_specs=vmem,
        scratch_shapes=[
            pltpu.VMEM((B, D), BF16),
            pltpu.VMEM((D,), BF16),
            pltpu.VMEM((B, NG, 2, GD, WH), BF16),
            pltpu.VMEM((B, NU, UD, W), BF16),
            pltpu.VMEM((NG, D, GD), BF16),
            pltpu.VMEM((HD, D), BF16),
            pltpu.VMEM((D, F), BF16),
            pltpu.VMEM((D, F), BF16),
            pltpu.VMEM((F, D), BF16),
            pltpu.VMEM((B, 8, D), F32),
            pltpu.VMEM((NG, G, GD), F32),
            pltpu.VMEM((NG, G, W), F32),
            pltpu.VMEM((NG, G, W), F32),
            pltpu.VMEM((8, D), F32),
            pltpu.SemaphoreType.DMA((B * NG * 2 + B * NU + 2 * NG + 5,)),
        ],
        compiler_params=pltpu.CompilerParams(vmem_limit_bytes=127 * 1024 * 1024),
    )(x2, B_w_r, kt, vt, A_wq, A_wo, B_w_gate, B_w_up, B_w_down)
    return out.reshape(B, Sq, D)
```

```python
import jax
import jax.numpy as jnp
from jax import lax
import jax.experimental.pallas as pl
import jax.experimental.pallas.tpu as pltpu

F32 = jnp.float32
BF16 = jnp.bfloat16
_HQ, _DH = 32, 192
OPT = dict(t7=1, scoped=1)


def _layernorm(x, eps=1e-5):
    m = jnp.mean(x, axis=-1, keepdims=True)
    xc = x - m
    v = jnp.mean(xc * xc, axis=-1, keepdims=True)
    return xc * lax.rsqrt(v + eps)


@jax.jit
def pallas_interleave_layers__sliding_block_cached__moe_arch_mod__decode_kernel(
    A_x, A_k_cache, A_v_cache, A_wq, A_wo, B_x, B_w_r, B_w_gate, B_w_up, B_w_down):
    del B_x
    B, Sq, D = A_x.shape
    _, Hkv, Sk, Dh = A_k_cache.shape
    F = B_w_gate.shape[1]
    W = min(4096, max(256, Sk // 4))
    HD = _HQ * _DH
    G = 8
    NG = _HQ // G
    GD = G * _DH
    NU = 2 * NG
    UD = HD // NU
    UH = UD // _DH
    HU = UD // 2
    NSEM = B * NG + B * (NU + 1) + NG + 3
    WH = W // 2
    NJ = W // 128
    scale = float(_DH) ** -0.5
    NT = (((1,), (1,)), ((), ()))

    def kernel(x_hbm, wr_hbm, k_hbm, v_hbm, wq_hbm, wo_hbm, wg_hbm, wu_hbm, wd_hbm,
               out_ref,
               xin, wr, kbuf, vbuf, wq, wo, wg, wu, wd, x_scr, q_scr, s_scr, p_scr, o_scr, osem):
        def body(sems):
            kernel_body(x_hbm, wr_hbm, k_hbm, v_hbm, wq_hbm, wo_hbm, wg_hbm, wu_hbm, wd_hbm,
                        xin, wr, kbuf, vbuf, wq, wo, wg, wu, wd, x_scr, q_scr, s_scr, p_scr, o_scr, sems)
            pltpu.make_async_copy(o_scr, out_ref, osem).start()
        pl.run_scoped(body, pltpu.SemaphoreType.DMA((NSEM,)))
        pltpu.make_async_copy(o_scr, out_ref, osem).wait()

    def kernel_body(x_hbm, wr_hbm, k_hbm, v_hbm, wq_hbm, wo_hbm, wg_hbm, wu_hbm, wd_hbm,
                    xin, wr, kbuf, vbuf, wq, wo, wg, wu, wd, x_scr, q_scr, s_scr, p_scr, o_scr, sems):
        KS = 0
        VS = B * NG
        WS = VS + B * (NU + 1)

        def k_copy(b, g, half):
            return pltpu.make_async_copy(
                k_hbm.at[b, pl.ds(g * GD, GD), pl.ds(Sk - W + half * WH, WH)],
                kbuf.at[b, g, half], sems.at[KS + b * NG + g])

        def v_copy(b, u):
            return pltpu.make_async_copy(
                v_hbm.at[b, pl.ds(u * UD, UD), pl.ds(Sk - W, W)],
                vbuf.at[b, u], sems.at[VS + b * (NU + 1) + u])

        def vlast_copy(b, h):
            return pltpu.make_async_copy(
                v_hbm.at[b, pl.ds((NU - 1) * UD + h * HU, HU), pl.ds(Sk - W, W)],
                vbuf.at[b, NU - 1, pl.ds(h * HU, HU)], sems.at[VS + b * (NU + 1) + NU - 1 + h])

        def wq_copy(g):
            return pltpu.make_async_copy(wq_hbm.at[:, pl.ds(g * GD, GD)], wq.at[g], sems.at[WS])

        def wo_copy(g):
            return pltpu.make_async_copy(wo_hbm.at[pl.ds(g * GD, GD), :], wo.at[pl.ds(g * GD, GD), :], sems.at[WS + 1 + g])

        small = [
            pltpu.make_async_copy(wg_hbm, wg, sems.at[WS + NG + 1]),
            pltpu.make_async_copy(wu_hbm, wu, sems.at[WS + NG + 1]),
            pltpu.make_async_copy(wd_hbm, wd, sems.at[WS + NG + 1]),
            pltpu.make_async_copy(x_hbm, xin, sems.at[WS + NG + 2]),
            pltpu.make_async_copy(wr_hbm, wr, sems.at[WS + NG + 2]),
        ]

        small[3].start()
        small[4].start()
        for g in range(NG):
            wq_copy(g).start()
        for g in range(NG):
            k_copy(0, g, 0).start()
            k_copy(0, g, 1).start()
        for u in range(NU - 1):
            v_copy(0, u).start()
            if u % 2 == 1:
                wo_copy(u // 2).start()
        wo_copy(NG - 1).start()
        vlast_copy(0, 0).start()
        vlast_copy(0, 1).start()
        for c in small[:3]:
            c.start()
        for b in range(1, B):
            for g in range(NG):
                k_copy(b, g, 0).start()
                k_copy(b, g, 1).start()
            for u in range(NU - 1):
                v_copy(b, u).start()
            vlast_copy(b, 0).start()
            vlast_copy(b, 1).start()

        small[3].wait()
        small[4].wait()
        x_in = xin[...].astype(F32)
        for b in range(B):
            x_scr[b] = jnp.broadcast_to(x_in[b:b + 1, :], (8, D))
        w_r = wr[...].astype(F32).reshape(1, D)

        row = lax.broadcasted_iota(jnp.int32, (G, GD), 0)
        col = lax.broadcasted_iota(jnp.int32, (G, GD), 1)
        diag = (col >= row * _DH) & (col < (row + 1) * _DH)
        diag_u = [diag[:, :UD], diag[:, UD:]]

        def transpose_unit(b, u, js=range(NJ)):
            for n in range(UD // 128):
                for j in js:
                    sl = (b, u, pl.ds(n * 128, 128), pl.ds(j * 128, 128))
                    vbuf[sl] = vbuf[sl].T

        def pv_xpose(b, u, pg):
            return lax.dot_general(pg, vbuf[b, u], NT, preferred_element_type=F32)

        def pv_plain(b, u, pg):
            outs = []
            for n in range(UD // 128):
                acc = None
                for j in range(NJ):
                    d = jnp.dot(pg[:, j * 128:(j + 1) * 128],
                                vbuf[b, u, pl.ds(n * 128, 128), pl.ds(j * 128, 128)],
                                preferred_element_type=F32)
                    acc = d if acc is None else acc + d
                outs.append(acc)
            return jnp.concatenate(outs, axis=1)

        def ffn(b, x, first):
            if first:
                @pl.when(b == 0)
                def _():
                    small[0].wait()
                    small[1].wait()
                    small[2].wait()
            xnb = _layernorm(x).astype(BF16)
            xnr = xnb.astype(F32)
            r = jnp.sum(xnr * w_r, axis=-1, keepdims=True)
            gate = jnp.dot(xnb, wg[...], preferred_element_type=F32)
            up = jnp.dot(xnb, wu[...], preferred_element_type=F32)
            h = (gate * jax.nn.sigmoid(gate) * up).astype(BF16)
            y = jnp.dot(h, wd[...], preferred_element_type=F32)
            return x + (xnr + y * jax.nn.sigmoid(r))

        def softmax():
            s = s_scr[...].reshape(NG * G, W) * scale
            m = jnp.max(s, axis=-1, keepdims=True)
            p = jnp.exp(s - m)
            l = jnp.sum(p, axis=-1, keepdims=True)
            p_scr[...] = (p / l).reshape(NG, G, W)

        def finish(o, u):
            return jnp.where(diag_u[u % 2], o, 0.0).astype(BF16)

        def layer1(b, x):
            xn = _layernorm(x).astype(BF16)
            @pl.when(b == 0)
            def _():
                for g in range(NG):
                    wq_copy(g).wait()

            def q_group(g, c):
                q_scr[g] = jnp.dot(xn, wq[g], preferred_element_type=F32)
                return c
            lax.fori_loop(0, NG, q_group, 0)
            def qk_group(g, c):
                qbd = jnp.where(diag, q_scr[g], 0.0).astype(BF16)
                k_copy(b, g, 0).wait()
                k_copy(b, g, 1).wait()
                for half in range(2):
                    s_scr[g, :, pl.ds(half * WH, WH)] = jnp.dot(
                        qbd, kbuf[b, g, half], preferred_element_type=F32)
                return c
            lax.fori_loop(0, NG, qk_group, 0)
            softmax()
            def unit(u2, acc):
                for r in range(2):
                    u = u2 * 2 + r

                    @pl.when(u > 0)
                    def _():
                        transpose_unit(b, u - 1)
                    v_copy(b, u).wait()
                    pg = p_scr[u2].astype(BF16)
                    o = finish(pv_xpose(b, u, pg), r)
                    if r == 0:
                        @pl.when(b == 0)
                        def _():
                            wo_copy(u2).wait()
                    acc = acc + jnp.dot(o, wo[pl.ds(pl.multiple_of(u * UD, UD), UD), :], preferred_element_type=F32)
                return acc
            acc = lax.fori_loop(0, NG - 1, unit, jnp.zeros((8, D), F32))
            pg = p_scr[NG - 1].astype(BF16)
            transpose_unit(b, NU - 3)
            v_copy(b, NU - 2).wait()
            o = finish(pv_xpose(b, NU - 2, pg), 0)

            @pl.when(b == 0)
            def _():
                wo_copy(NG - 1).wait()
            acc = acc + jnp.dot(o, wo[pl.ds((NU - 2) * UD, UD), :], preferred_element_type=F32)
            transpose_unit(b, NU - 2)
            for h in range(2):
                vlast_copy(b, h).wait()
                o = lax.dot_general(pg, vbuf[b, NU - 1, pl.ds(h * HU, HU), :], NT, preferred_element_type=F32)
                o = jnp.where(diag_u[1][:, h * HU:(h + 1) * HU], o, 0.0).astype(BF16)
                acc = acc + jnp.dot(o, wo[pl.ds((NU - 1) * UD + h * HU, HU), :], preferred_element_type=F32)
            return x + jnp.sum(acc, axis=0, keepdims=True)

        def layer2(b, x):
            xn = _layernorm(x).astype(BF16)
            for g in range(NG):
                q_scr[g] = jnp.dot(xn, wq[g], preferred_element_type=F32)
                if OPT["t7"]:
                    transpose_unit(b, NU - 1, range(2 * g, 2 * g + 2))
            for g in range(NG):
                qbd = jnp.where(diag, q_scr[g], 0.0).astype(BF16)
                for half in range(2):
                    s_scr[g, :, pl.ds(half * WH, WH)] = jnp.dot(
                        qbd, kbuf[b, g, half], preferred_element_type=F32)
            softmax()
            os_ = []
            for u in range(NU):
                pg = p_scr[u // 2].astype(BF16)
                o = pv_plain(b, u, pg) if (u < NU - 1 or OPT['t7']) else pv_xpose(b, u, pg)
                os_.append(finish(o, u))
            ocat = jnp.concatenate(os_, axis=1)
            acc = jnp.dot(ocat, wo[...], preferred_element_type=F32)
            return x + jnp.sum(acc, axis=0, keepdims=True)

        def batch(b, carry):
            x = x_scr[b]
            x = layer1(b, x)
            x = ffn(b, x, True)
            x = layer2(b, x)
            x = ffn(b, x, False)
            x_scr[b] = x
            return carry

        lax.fori_loop(0, B, batch, 0)

        out = jnp.concatenate([x_scr[b][0:1, :] for b in range(B)], axis=0)
        o_scr[...] = out.astype(o_scr.dtype)

    kt = jnp.transpose(A_k_cache, (0, 1, 3, 2)).reshape(B, HD, Sk)
    vt = jnp.transpose(A_v_cache, (0, 1, 3, 2)).reshape(B, HD, Sk)
    x2 = A_x.reshape(B, D)

    hbm = pl.BlockSpec(memory_space=pltpu.HBM)
    out = pl.pallas_call(
        kernel,
        out_shape=jax.ShapeDtypeStruct((B, D), A_x.dtype),
        in_specs=[hbm] * 9,
        out_specs=hbm,
        scratch_shapes=[
            pltpu.VMEM((B, D), BF16),
            pltpu.VMEM((D,), BF16),
            pltpu.VMEM((B, NG, 2, GD, WH), BF16),
            pltpu.VMEM((B, NU, UD, W), BF16),
            pltpu.VMEM((NG, D, GD), BF16),
            pltpu.VMEM((HD, D), BF16),
            pltpu.VMEM((D, F), BF16),
            pltpu.VMEM((D, F), BF16),
            pltpu.VMEM((F, D), BF16),
            pltpu.VMEM((B, 8, D), F32),
            pltpu.VMEM((NG, G, GD), F32),
            pltpu.VMEM((NG, G, W), F32),
            pltpu.VMEM((NG, G, W), F32),
            pltpu.VMEM((B, D), BF16),
            pltpu.SemaphoreType.DMA(()),
        ],
        compiler_params=pltpu.CompilerParams(vmem_limit_bytes=127 * 1024 * 1024),
    )(x2, B_w_r, kt, vt, A_wq, A_wo, B_w_gate, B_w_up, B_w_down)
    return out.reshape(B, Sq, D)
```

```python
import jax
import jax.numpy as jnp
from jax import lax
import jax.experimental.pallas as pl
import jax.experimental.pallas.tpu as pltpu

F32 = jnp.float32
BF16 = jnp.bfloat16
_HQ, _DH = 32, 192
OPT = dict(t7=1, ln1=1)


def _layernorm(x, eps=1e-5):
    m = jnp.mean(x, axis=-1, keepdims=True)
    if OPT["ln1"]:
        v = jnp.maximum(jnp.mean(x * x, axis=-1, keepdims=True) - m * m, 0.0)
        return (x - m) * lax.rsqrt(v + eps)
    xc = x - m
    v = jnp.mean(xc * xc, axis=-1, keepdims=True)
    return xc * lax.rsqrt(v + eps)


@jax.jit
def pallas_interleave_layers__sliding_block_cached__moe_arch_mod__decode_kernel(
    A_x, A_k_cache, A_v_cache, A_wq, A_wo, B_x, B_w_r, B_w_gate, B_w_up, B_w_down):
    del B_x
    B, Sq, D = A_x.shape
    _, Hkv, Sk, Dh = A_k_cache.shape
    F = B_w_gate.shape[1]
    W = min(4096, max(256, Sk // 4))
    HD = _HQ * _DH
    G = 8
    NG = _HQ // G
    GD = G * _DH
    NU = 2 * NG
    UD = HD // NU
    UH = UD // _DH
    HU = UD // 2
    NSEM = B + (B - 1) * NG + NU + 1 + 4
    WH = W // 2
    NJ = W // 128
    scale = float(_DH) ** -0.5
    NT = (((1,), (1,)), ((), ()))

    def kernel(x_hbm, wr_hbm, k_hbm, v_hbm, wq_hbm, wo_hbm, wg_hbm, wu_hbm, wd_hbm,
               out_ref,
               xin, wr, kbuf, vbuf, wq, wo, wg, wu, wd, x_scr, q_scr, s_scr, p_scr, o_scr, osem):
        def body(sems):
            kernel_body(x_hbm, wr_hbm, k_hbm, v_hbm, wq_hbm, wo_hbm, wg_hbm, wu_hbm, wd_hbm,
                        xin, wr, kbuf, vbuf, wq, wo, wg, wu, wd, x_scr, q_scr, s_scr, p_scr, o_scr, sems)
            pltpu.make_async_copy(o_scr, out_ref, osem).start()
        pl.run_scoped(body, pltpu.SemaphoreType.DMA((NSEM,)))
        pltpu.make_async_copy(o_scr, out_ref, osem).wait()

    def kernel_body(x_hbm, wr_hbm, k_hbm, v_hbm, wq_hbm, wo_hbm, wg_hbm, wu_hbm, wd_hbm,
                    xin, wr, kbuf, vbuf, wq, wo, wg, wu, wd, x_scr, q_scr, s_scr, p_scr, o_scr, sems):
        KS = 0
        VS = B
        VL = VS + (B - 1) * NG
        WS = VL + NU + 1

        def k_copy(b, half):
            return pltpu.make_async_copy(
                k_hbm.at[b, :, pl.ds(Sk - W + half * WH, WH)], kbuf.at[b, half], sems.at[KS + b])

        def vgroup_copy(b, g):
            return pltpu.make_async_copy(
                v_hbm.at[b, pl.ds(2 * g, 2), :, pl.ds(Sk - W, W)],
                vbuf.at[b, pl.ds(2 * g, 2)], sems.at[VS + b * NG + g])

        def v_copy(u):
            return pltpu.make_async_copy(
                v_hbm.at[B - 1, u, :, pl.ds(Sk - W, W)], vbuf.at[B - 1, u], sems.at[VL + u])

        def vlast_copy(h):
            return pltpu.make_async_copy(
                v_hbm.at[B - 1, NU - 1, pl.ds(h * HU, HU), pl.ds(Sk - W, W)],
                vbuf.at[B - 1, NU - 1, pl.ds(h * HU, HU)], sems.at[VL + NU - 1 + h])

        def wq_copy(g):
            return pltpu.make_async_copy(wq_hbm.at[:, pl.ds(g * GD, GD)], wq.at[g], sems.at[WS])

        wo_copy = pltpu.make_async_copy(wo_hbm, wo, sems.at[WS + 1])

        small = [
            pltpu.make_async_copy(wg_hbm, wg, sems.at[WS + 2]),
            pltpu.make_async_copy(wu_hbm, wu, sems.at[WS + 2]),
            pltpu.make_async_copy(wd_hbm, wd, sems.at[WS + 2]),
            pltpu.make_async_copy(x_hbm, xin, sems.at[WS + 3]),
            pltpu.make_async_copy(wr_hbm, wr, sems.at[WS + 3]),
        ]

        small[3].start()
        small[4].start()
        for g in range(NG):
            wq_copy(g).start()
        k_copy(0, 0).start()
        k_copy(0, 1).start()
        wo_copy.start()
        for g in range(NG):
            vgroup_copy(0, g).start()
        for c in small[:3]:
            c.start()
        for b in range(1, B):
            k_copy(b, 0).start()
            k_copy(b, 1).start()
            if b < B - 1:
                for g in range(NG):
                    vgroup_copy(b, g).start()
        for u in range(NU - 1):
            v_copy(u).start()
        vlast_copy(0).start()
        vlast_copy(1).start()

        small[3].wait()
        small[4].wait()
        x_in = xin[...].astype(F32)
        for b in range(B):
            x_scr[b] = jnp.broadcast_to(x_in[b:b + 1, :], (8, D))
        w_r = wr[...].astype(F32).reshape(1, D)

        row = lax.broadcasted_iota(jnp.int32, (G, GD), 0)
        col = lax.broadcasted_iota(jnp.int32, (G, GD), 1)
        diag = (col >= row * _DH) & (col < (row + 1) * _DH)
        diag_u = [diag[:, :UD], diag[:, UD:]]

        def transpose_unit(b, u, js=range(NJ)):
            for n in range(UD // 128):
                for j in js:
                    sl = (b, u, pl.ds(n * 128, 128), pl.ds(j * 128, 128))
                    vbuf[sl] = vbuf[sl].T

        def pv_xpose(b, u, pg):
            return lax.dot_general(pg, vbuf[b, u], NT, preferred_element_type=F32)

        def pv_plain(b, u, pg):
            outs = []
            for n in range(UD // 128):
                acc = None
                for j in range(NJ):
                    d = jnp.dot(pg[:, j * 128:(j + 1) * 128],
                                vbuf[b, u, pl.ds(n * 128, 128), pl.ds(j * 128, 128)],
                                preferred_element_type=F32)
                    acc = d if acc is None else acc + d
                outs.append(acc)
            return jnp.concatenate(outs, axis=1)

        def ffn(b, x, first):
            if first:
                @pl.when(b == 0)
                def _():
                    small[0].wait()
                    small[1].wait()
                    small[2].wait()
            xnb = _layernorm(x).astype(BF16)
            xnr = xnb.astype(F32)
            r = jnp.sum(xnr * w_r, axis=-1, keepdims=True)
            gate = jnp.dot(xnb, wg[...], preferred_element_type=F32)
            up = jnp.dot(xnb, wu[...], preferred_element_type=F32)
            h = (gate * jax.nn.sigmoid(gate) * up).astype(BF16)
            y = jnp.dot(h, wd[...], preferred_element_type=F32)
            return x + (xnr + y * jax.nn.sigmoid(r))

        def softmax():
            s = s_scr[...].reshape(NG * G, W) * scale
            m = jnp.max(s, axis=-1, keepdims=True)
            p = jnp.exp(s - m)
            l = jnp.sum(p, axis=-1, keepdims=True)
            p_scr[...] = (p / l).reshape(NG, G, W)

        def finish(o, u):
            return jnp.where(diag_u[u % 2], o, 0.0).astype(BF16)

        def layer1(b, x):
            xn = _layernorm(x).astype(BF16)
            @pl.when(b == 0)
            def _():
                for g in range(NG):
                    wq_copy(g).wait()

            def q_group(g, c):
                q_scr[g] = jnp.dot(xn, wq[g], preferred_element_type=F32)
                return c
            lax.fori_loop(0, NG, q_group, 0)
            k_copy(b, 0).wait()
            k_copy(b, 1).wait()
            def qk_group(g, c):
                qbd = jnp.where(diag, q_scr[g], 0.0).astype(BF16)
                for half in range(2):
                    s_scr[g, :, pl.ds(half * WH, WH)] = jnp.dot(
                        qbd, kbuf[b, half, pl.ds(pl.multiple_of(g * GD, GD), GD), :], preferred_element_type=F32)
                return c
            lax.fori_loop(0, NG, qk_group, 0)
            softmax()
            def unit(u2, acc):
                for r in range(2):
                    u = u2 * 2 + r

                    @pl.when(u > 0)
                    def _():
                        transpose_unit(b, u - 1)
                    if r == 0:
                        @pl.when(b < B - 1)
                        def _():
                            vgroup_copy(b, u2).wait()

                    @pl.when(b == B - 1)
                    def _():
                        v_copy(u).wait()
                    pg = p_scr[u2].astype(BF16)
                    o = finish(pv_xpose(b, u, pg), r)
                    acc = acc + jnp.dot(o, wo[pl.ds(pl.multiple_of(u * UD, UD), UD), :], preferred_element_type=F32)
                return acc
            @pl.when(b == 0)
            def _():
                wo_copy.wait()
            acc = lax.fori_loop(0, NG - 1, unit, jnp.zeros((8, D), F32))
            pg = p_scr[NG - 1].astype(BF16)
            transpose_unit(b, NU - 3)

            @pl.when(b < B - 1)
            def _():
                vgroup_copy(b, NG - 1).wait()

            @pl.when(b == B - 1)
            def _():
                v_copy(NU - 2).wait()
            o = finish(pv_xpose(b, NU - 2, pg), 0)
            acc = acc + jnp.dot(o, wo[pl.ds((NU - 2) * UD, UD), :], preferred_element_type=F32)
            transpose_unit(b, NU - 2)
            for h in range(2):
                @pl.when(b == B - 1)
                def _():
                    vlast_copy(h).wait()
                o = lax.dot_general(pg, vbuf[b, NU - 1, pl.ds(h * HU, HU), :], NT, preferred_element_type=F32)
                o = jnp.where(diag_u[1][:, h * HU:(h + 1) * HU], o, 0.0).astype(BF16)
                acc = acc + jnp.dot(o, wo[pl.ds((NU - 1) * UD + h * HU, HU), :], preferred_element_type=F32)
            return x + jnp.sum(acc, axis=0, keepdims=True)

        def layer2(b, x):
            xn = _layernorm(x).astype(BF16)
            for g in range(NG):
                q_scr[g] = jnp.dot(xn, wq[g], preferred_element_type=F32)
                if OPT["t7"]:
                    transpose_unit(b, NU - 1, range(2 * g, 2 * g + 2))
            for g in range(NG):
                qbd = jnp.where(diag, q_scr[g], 0.0).astype(BF16)
                for half in range(2):
                    s_scr[g, :, pl.ds(half * WH, WH)] = jnp.dot(
                        qbd, kbuf[b, half, pl.ds(g * GD, GD), :], preferred_element_type=F32)
            softmax()
            os_ = []
            for u in range(NU):
                pg = p_scr[u // 2].astype(BF16)
                o = pv_plain(b, u, pg) if (u < NU - 1 or OPT['t7']) else pv_xpose(b, u, pg)
                os_.append(finish(o, u))
            ocat = jnp.concatenate(os_, axis=1)
            acc = jnp.dot(ocat, wo[...], preferred_element_type=F32)
            return x + jnp.sum(acc, axis=0, keepdims=True)

        def batch(b, carry):
            x = x_scr[b]
            x = layer1(b, x)
            x = ffn(b, x, True)
            x = layer2(b, x)
            x = ffn(b, x, False)
            x_scr[b] = x
            return carry

        lax.fori_loop(0, B, batch, 0)

        out = jnp.concatenate([x_scr[b][0:1, :] for b in range(B)], axis=0)
        o_scr[...] = out.astype(o_scr.dtype)

    kt = jnp.transpose(A_k_cache, (0, 1, 3, 2)).reshape(B, HD, Sk)
    vt = jnp.transpose(A_v_cache, (0, 1, 3, 2)).reshape(B, NU, UD, Sk)
    x2 = A_x.reshape(B, D)

    hbm = pl.BlockSpec(memory_space=pltpu.HBM)
    out = pl.pallas_call(
        kernel,
        out_shape=jax.ShapeDtypeStruct((B, D), A_x.dtype),
        in_specs=[hbm] * 9,
        out_specs=hbm,
        scratch_shapes=[
            pltpu.VMEM((B, D), BF16),
            pltpu.VMEM((D,), BF16),
            pltpu.VMEM((B, 2, HD, WH), BF16),
            pltpu.VMEM((B, NU, UD, W), BF16),
            pltpu.VMEM((NG, D, GD), BF16),
            pltpu.VMEM((HD, D), BF16),
            pltpu.VMEM((D, F), BF16),
            pltpu.VMEM((D, F), BF16),
            pltpu.VMEM((F, D), BF16),
            pltpu.VMEM((B, 8, D), F32),
            pltpu.VMEM((NG, G, GD), F32),
            pltpu.VMEM((NG, G, W), F32),
            pltpu.VMEM((NG, G, W), F32),
            pltpu.VMEM((B, D), BF16),
            pltpu.SemaphoreType.DMA(()),
        ],
        compiler_params=pltpu.CompilerParams(vmem_limit_bytes=127 * 1024 * 1024),
    )(x2, B_w_r, kt, vt, A_wq, A_wo, B_w_gate, B_w_up, B_w_down)
    return out.reshape(B, Sq, D)
```

```python
import jax
import jax.numpy as jnp
from jax import lax
import jax.experimental.pallas as pl
import jax.experimental.pallas.tpu as pltpu

F32 = jnp.float32
BF16 = jnp.bfloat16
_HQ, _DH = 32, 192
OPT = dict(t7=1, ln1=1, last=1, out2=1)


def _layernorm(x, eps=1e-5):
    m = jnp.mean(x, axis=-1, keepdims=True)
    if OPT["ln1"]:
        v = jnp.maximum(jnp.mean(x * x, axis=-1, keepdims=True) - m * m, 0.0)
        return (x - m) * lax.rsqrt(v + eps)
    xc = x - m
    v = jnp.mean(xc * xc, axis=-1, keepdims=True)
    return xc * lax.rsqrt(v + eps)


@jax.jit
def pallas_interleave_layers__sliding_block_cached__moe_arch_mod__decode_kernel(
    A_x, A_k_cache, A_v_cache, A_wq, A_wo, B_x, B_w_r, B_w_gate, B_w_up, B_w_down):
    del B_x
    B, Sq, D = A_x.shape
    _, Hkv, Sk, Dh = A_k_cache.shape
    F = B_w_gate.shape[1]
    W = min(4096, max(256, Sk // 4))
    HD = _HQ * _DH
    G = 8
    NG = _HQ // G
    GD = G * _DH
    NU = 2 * NG
    UD = HD // NU
    UH = UD // _DH
    LAST = {0: [(0, 384), (384, 384)], 1: [(0, 384), (384, 256), (640, 128)], 2: [(0, 256), (256, 256), (512, 128), (640, 128)]}[OPT['last']]
    NSEM = B + (B - 1) * NG + NU - 1 + len(LAST) + 4
    WH = W // 2
    NJ = W // 128
    scale = float(_DH) ** -0.5
    NT = (((1,), (1,)), ((), ()))

    def kernel(x_hbm, wr_hbm, k_hbm, v_hbm, wq_hbm, wo_hbm, wg_hbm, wu_hbm, wd_hbm,
               out_ref,
               xin, wr, kbuf, vbuf, wq, wo, wg, wu, wd, x_scr, q_scr, s_scr, p_scr, o_scr, res_scr, osem):
        def body(sems):
            kernel_body(x_hbm, wr_hbm, k_hbm, v_hbm, wq_hbm, wo_hbm, wg_hbm, wu_hbm, wd_hbm,
                        xin, wr, kbuf, vbuf, wq, wo, wg, wu, wd, x_scr, q_scr, s_scr, p_scr, o_scr, res_scr, sems)
            pltpu.make_async_copy(o_scr, out_ref, osem).start()
        pl.run_scoped(body, pltpu.SemaphoreType.DMA((NSEM,)))
        pltpu.make_async_copy(o_scr, out_ref, osem).wait()

    def kernel_body(x_hbm, wr_hbm, k_hbm, v_hbm, wq_hbm, wo_hbm, wg_hbm, wu_hbm, wd_hbm,
                    xin, wr, kbuf, vbuf, wq, wo, wg, wu, wd, x_scr, q_scr, s_scr, p_scr, o_scr, res_scr, sems):
        KS = 0
        VS = B
        VL = VS + (B - 1) * NG
        WS = VL + NU - 1 + len(LAST)

        def k_copy(b, half):
            return pltpu.make_async_copy(
                k_hbm.at[b, :, pl.ds(Sk - W + half * WH, WH)], kbuf.at[b, half], sems.at[KS + b])

        def vgroup_copy(b, g):
            return pltpu.make_async_copy(
                v_hbm.at[b, pl.ds(2 * g, 2), :, pl.ds(Sk - W, W)],
                vbuf.at[b, pl.ds(2 * g, 2)], sems.at[VS + b * NG + g])

        def v_copy(u):
            return pltpu.make_async_copy(
                v_hbm.at[B - 1, u, :, pl.ds(Sk - W, W)], vbuf.at[B - 1, u], sems.at[VL + u])

        def vlast_copy(h):
            r0, nr = LAST[h]
            return pltpu.make_async_copy(
                v_hbm.at[B - 1, NU - 1, pl.ds(r0, nr), pl.ds(Sk - W, W)],
                vbuf.at[B - 1, NU - 1, pl.ds(r0, nr)], sems.at[VL + NU - 1 + h])

        def wq_copy(g):
            return pltpu.make_async_copy(wq_hbm.at[:, pl.ds(g * GD, GD)], wq.at[g], sems.at[WS])

        wo_copy = pltpu.make_async_copy(wo_hbm, wo, sems.at[WS + 1])

        small = [
            pltpu.make_async_copy(wg_hbm, wg, sems.at[WS + 2]),
            pltpu.make_async_copy(wu_hbm, wu, sems.at[WS + 2]),
            pltpu.make_async_copy(wd_hbm, wd, sems.at[WS + 2]),
            pltpu.make_async_copy(x_hbm, xin, sems.at[WS + 3]),
            pltpu.make_async_copy(wr_hbm, wr, sems.at[WS + 3]),
        ]

        small[3].start()
        small[4].start()
        for g in range(NG):
            wq_copy(g).start()
        k_copy(0, 0).start()
        k_copy(0, 1).start()
        wo_copy.start()
        for g in range(NG):
            vgroup_copy(0, g).start()
        for c in small[:3]:
            c.start()
        for b in range(1, B):
            k_copy(b, 0).start()
            k_copy(b, 1).start()
            if b < B - 1:
                for g in range(NG):
                    vgroup_copy(b, g).start()
        for u in range(NU - 1):
            v_copy(u).start()
        for h in range(len(LAST)):
            vlast_copy(h).start()

        small[3].wait()
        small[4].wait()
        x_in = xin[...].astype(F32)
        for b in range(B):
            x_scr[b] = jnp.broadcast_to(x_in[b:b + 1, :], (8, D))
        w_r = wr[...].astype(F32).reshape(1, D)
        res_scr[...] = jnp.zeros((8, D), F32)

        row = lax.broadcasted_iota(jnp.int32, (G, GD), 0)
        col = lax.broadcasted_iota(jnp.int32, (G, GD), 1)
        diag = (col >= row * _DH) & (col < (row + 1) * _DH)
        diag_u = [diag[:, :UD], diag[:, UD:]]

        def transpose_unit(b, u, js=range(NJ)):
            for n in range(UD // 128):
                for j in js:
                    sl = (b, u, pl.ds(n * 128, 128), pl.ds(j * 128, 128))
                    vbuf[sl] = vbuf[sl].T

        def pv_xpose(b, u, pg):
            return lax.dot_general(pg, vbuf[b, u], NT, preferred_element_type=F32)

        def pv_plain(b, u, pg):
            outs = []
            for n in range(UD // 128):
                acc = None
                for j in range(NJ):
                    d = jnp.dot(pg[:, j * 128:(j + 1) * 128],
                                vbuf[b, u, pl.ds(n * 128, 128), pl.ds(j * 128, 128)],
                                preferred_element_type=F32)
                    acc = d if acc is None else acc + d
                outs.append(acc)
            return jnp.concatenate(outs, axis=1)

        def ffn(b, x, first):
            if first:
                @pl.when(b == 0)
                def _():
                    small[0].wait()
                    small[1].wait()
                    small[2].wait()
            xnb = _layernorm(x).astype(BF16)
            xnr = xnb.astype(F32)
            r = jnp.sum(xnr * w_r, axis=-1, keepdims=True)
            gate = jnp.dot(xnb, wg[...], preferred_element_type=F32)
            up = jnp.dot(xnb, wu[...], preferred_element_type=F32)
            h = (gate * jax.nn.sigmoid(gate) * up).astype(BF16)
            y = jnp.dot(h, wd[...], preferred_element_type=F32)
            return x + (xnr + y * jax.nn.sigmoid(r))

        def softmax():
            s = s_scr[...].reshape(NG * G, W) * scale
            m = jnp.max(s, axis=-1, keepdims=True)
            p = jnp.exp(s - m)
            l = jnp.sum(p, axis=-1, keepdims=True)
            p_scr[...] = (p / l).reshape(NG, G, W)

        def finish(o, u):
            return jnp.where(diag_u[u % 2], o, 0.0).astype(BF16)

        def layer1(b, x):
            xn = _layernorm(x).astype(BF16)
            @pl.when(b == 0)
            def _():
                for g in range(NG):
                    wq_copy(g).wait()

            def q_group(g, c):
                q_scr[g] = jnp.dot(xn, wq[g], preferred_element_type=F32)
                return c
            lax.fori_loop(0, NG, q_group, 0)
            k_copy(b, 0).wait()
            k_copy(b, 1).wait()
            def qk_group(g, c):
                qbd = jnp.where(diag, q_scr[g], 0.0).astype(BF16)
                for half in range(2):
                    s_scr[g, :, pl.ds(half * WH, WH)] = jnp.dot(
                        qbd, kbuf[b, half, pl.ds(pl.multiple_of(g * GD, GD), GD), :], preferred_element_type=F32)
                return c
            lax.fori_loop(0, NG, qk_group, 0)
            softmax()
            def unit(u2, acc):
                for r in range(2):
                    u = u2 * 2 + r

                    @pl.when(u > 0)
                    def _():
                        transpose_unit(b, u - 1)
                    if r == 0:
                        @pl.when(b < B - 1)
                        def _():
                            vgroup_copy(b, u2).wait()

                    @pl.when(b == B - 1)
                    def _():
                        v_copy(u).wait()
                    pg = p_scr[u2].astype(BF16)
                    o = finish(pv_xpose(b, u, pg), r)
                    acc = acc + jnp.dot(o, wo[pl.ds(pl.multiple_of(u * UD, UD), UD), :], preferred_element_type=F32)
                return acc
            @pl.when(b == 0)
            def _():
                wo_copy.wait()
            acc = lax.fori_loop(0, NG - 1, unit, jnp.zeros((8, D), F32))
            pg = p_scr[NG - 1].astype(BF16)
            transpose_unit(b, NU - 3)

            @pl.when(b < B - 1)
            def _():
                vgroup_copy(b, NG - 1).wait()

            @pl.when(b == B - 1)
            def _():
                v_copy(NU - 2).wait()
            o = finish(pv_xpose(b, NU - 2, pg), 0)
            acc = acc + jnp.dot(o, wo[pl.ds((NU - 2) * UD, UD), :], preferred_element_type=F32)
            transpose_unit(b, NU - 2)
            for h, (r0, nr) in enumerate(LAST):
                @pl.when(b == B - 1)
                def _():
                    vlast_copy(h).wait()
                o = lax.dot_general(pg, vbuf[b, NU - 1, pl.ds(r0, nr), :], NT, preferred_element_type=F32)
                o = jnp.where(diag_u[1][:, r0:r0 + nr], o, 0.0).astype(BF16)
                acc = acc + jnp.dot(o, wo[pl.ds((NU - 1) * UD + r0, nr), :], preferred_element_type=F32)
            return x + jnp.sum(acc, axis=0, keepdims=True)

        def layer2(b, x):
            xn = _layernorm(x).astype(BF16)
            for g in range(NG):
                q_scr[g] = jnp.dot(xn, wq[g], preferred_element_type=F32)
                if OPT["t7"]:
                    transpose_unit(b, NU - 1, range(2 * g, 2 * g + 2))
            for g in range(NG):
                qbd = jnp.where(diag, q_scr[g], 0.0).astype(BF16)
                for half in range(2):
                    s_scr[g, :, pl.ds(half * WH, WH)] = jnp.dot(
                        qbd, kbuf[b, half, pl.ds(g * GD, GD), :], preferred_element_type=F32)
            softmax()
            os_ = []
            for u in range(NU):
                pg = p_scr[u // 2].astype(BF16)
                o = pv_plain(b, u, pg) if (u < NU - 1 or OPT['t7']) else pv_xpose(b, u, pg)
                os_.append(finish(o, u))
            ocat = jnp.concatenate(os_, axis=1)
            acc = jnp.dot(ocat, wo[...], preferred_element_type=F32)
            return x + jnp.sum(acc, axis=0, keepdims=True)

        def batch(b, carry):
            x = x_scr[b]
            x = layer1(b, x)
            x = ffn(b, x, True)
            x = layer2(b, x)
            x = ffn(b, x, False)
            if OPT["out2"]:
                rows = lax.broadcasted_iota(jnp.int32, (8, D), 0)
                res = jnp.where(rows == b, x, res_scr[...])
                res_scr[...] = res
                o_scr[...] = res[0:B].astype(o_scr.dtype)
            else:
                x_scr[b] = x
            return carry

        lax.fori_loop(0, B, batch, 0)

        if not OPT["out2"]:
            out = jnp.concatenate([x_scr[b][0:1, :] for b in range(B)], axis=0)
            o_scr[...] = out.astype(o_scr.dtype)

    kt = jnp.transpose(A_k_cache, (0, 1, 3, 2)).reshape(B, HD, Sk)
    vt = jnp.transpose(A_v_cache, (0, 1, 3, 2)).reshape(B, NU, UD, Sk)
    x2 = A_x.reshape(B, D)

    hbm = pl.BlockSpec(memory_space=pltpu.HBM)
    out = pl.pallas_call(
        kernel,
        out_shape=jax.ShapeDtypeStruct((B, D), A_x.dtype),
        in_specs=[hbm] * 9,
        out_specs=hbm,
        scratch_shapes=[
            pltpu.VMEM((B, D), BF16),
            pltpu.VMEM((D,), BF16),
            pltpu.VMEM((B, 2, HD, WH), BF16),
            pltpu.VMEM((B, NU, UD, W), BF16),
            pltpu.VMEM((NG, D, GD), BF16),
            pltpu.VMEM((HD, D), BF16),
            pltpu.VMEM((D, F), BF16),
            pltpu.VMEM((D, F), BF16),
            pltpu.VMEM((F, D), BF16),
            pltpu.VMEM((B, 8, D), F32),
            pltpu.VMEM((NG, G, GD), F32),
            pltpu.VMEM((NG, G, W), F32),
            pltpu.VMEM((NG, G, W), F32),
            pltpu.VMEM((B, D), BF16),
            pltpu.VMEM((8, D), F32),
            pltpu.SemaphoreType.DMA(()),
        ],
        compiler_params=pltpu.CompilerParams(vmem_limit_bytes=127 * 1024 * 1024),
    )(x2, B_w_r, kt, vt, A_wq, A_wo, B_w_gate, B_w_up, B_w_down)
    return out.reshape(B, Sq, D)
```

```python
import jax
import jax.numpy as jnp
from jax import lax
import jax.experimental.pallas as pl
import jax.experimental.pallas.tpu as pltpu


F32 = jnp.float32
BF16 = jnp.bfloat16
_HQ, _DH = 32, 192
_NT = (((1,), (1,)), ((), ()))


def _layernorm(x, eps=1e-5):
    m = jnp.mean(x, axis=-1, keepdims=True)
    v = jnp.maximum(jnp.mean(x * x, axis=-1, keepdims=True) - m * m, 0.0)
    return (x - m) * lax.rsqrt(v + eps)


def _bcast_sum(a):
    return jnp.broadcast_to(jnp.sum(a, axis=0, keepdims=True), a.shape)


def _columns(rowvec):
    return jnp.broadcast_to(rowvec, (128, rowvec.shape[1])).T


@jax.jit
def pallas_interleave_layers__sliding_block_cached__moe_arch_mod__decode_kernel(
    A_x: jax.Array,
    A_k_cache: jax.Array,
    A_v_cache: jax.Array,
    A_wq: jax.Array,
    A_wo: jax.Array,
    B_x: jax.Array,
    B_w_r: jax.Array,
    B_w_gate: jax.Array,
    B_w_up: jax.Array,
    B_w_down: jax.Array,
):
    del B_x
    B, Sq, D = A_x.shape
    _, Hkv, Sk, Dh = A_k_cache.shape
    assert Sq == 1 and Hkv == _HQ and Dh == _DH
    F = B_w_gate.shape[1]
    W = min(4096, max(256, Sk // 4))
    HD = _HQ * _DH
    G = 8
    NG = _HQ // G
    GD = G * _DH
    NU = 2 * NG
    UD = HD // NU
    WH = W // 2
    NJ = W // 128
    NTF = F // 128
    LAST = ((0, 384), (384, 256), (640, 128))
    KV = 128
    NV = 2
    scale = float(_DH) ** -0.5

    KS = 0
    VS = KS + B
    VL = VS + (B - 1) * NG
    WS = VL + NU - 1 + len(LAST)
    NSEM = WS + 4

    def body(x_hbm, wr_hbm, k_hbm, v_hbm, wq_hbm, wo_hbm, wg_hbm, wu_hbm, wd_hbm,
             xin, wr, kbuf, vbuf, wq, wo, wg, wu, wd,
             x_scr, q_scr, s_scr, p_scr, xcol, res_scr, o_scr, sems):

        def k_copy(b, half):
            return pltpu.make_async_copy(
                k_hbm.at[b, :, pl.ds(Sk - W + half * WH, WH)], kbuf.at[b, half], sems.at[KS + b])

        def vgroup_copy(b, g):
            return pltpu.make_async_copy(
                v_hbm.at[b, pl.ds(2 * g, 2), :, pl.ds(Sk - W, W)],
                vbuf.at[b, pl.ds(2 * g, 2)], sems.at[VS + b * NG + g])

        def vunit_copy(u):
            return pltpu.make_async_copy(
                v_hbm.at[B - 1, u, :, pl.ds(Sk - W, W)], vbuf.at[B - 1, u], sems.at[VL + u])

        def vlast_copy(h):
            r0, nr = LAST[h]
            return pltpu.make_async_copy(
                v_hbm.at[B - 1, NU - 1, pl.ds(r0, nr), pl.ds(Sk - W, W)],
                vbuf.at[B - 1, NU - 1, pl.ds(r0, nr)], sems.at[VL + NU - 1 + h])

        wq_copies = [pltpu.make_async_copy(wq_hbm.at[:, pl.ds(g * GD, GD)], wq.at[g], sems.at[WS])
                     for g in range(NG)]
        wo_copy = pltpu.make_async_copy(wo_hbm, wo, sems.at[WS + 1])
        ffn_copies = [pltpu.make_async_copy(s, d, sems.at[WS + 2])
                      for s, d in ((wg_hbm, wg), (wu_hbm, wu), (wd_hbm, wd))]
        row_copies = [pltpu.make_async_copy(x_hbm, xin, sems.at[WS + 3]),
                      pltpu.make_async_copy(wr_hbm, wr, sems.at[WS + 3])]

        for c in row_copies + wq_copies:
            c.start()
        k_copy(0, 0).start()
        k_copy(0, 1).start()
        wo_copy.start()
        for g in range(NG):
            vgroup_copy(0, g).start()
        for c in ffn_copies:
            c.start()
        for b in range(1, B):
            k_copy(b, 0).start()
            k_copy(b, 1).start()
            if b < B - 1:
                for g in range(NG):
                    vgroup_copy(b, g).start()
        for u in range(NU - 1):
            vunit_copy(u).start()
        for h in range(len(LAST)):
            vlast_copy(h).start()

        for c in row_copies:
            c.wait()
        x_in = xin[...].astype(F32)
        for b in range(B):
            x_scr[b] = jnp.broadcast_to(x_in[b:b + 1, :], (8, D))
        w_r = wr[...].astype(F32).reshape(1, D)
        res_scr[...] = jnp.zeros((8, D), F32)

        row = lax.broadcasted_iota(jnp.int32, (G, GD), 0)
        col = lax.broadcasted_iota(jnp.int32, (G, GD), 1)
        diag = (col >= row * _DH) & (col < (row + 1) * _DH)
        diag_u = [diag[:, :UD], diag[:, UD:]]

        def transpose_unit(b, u, js=range(NJ)):
            for n in range(UD // 128):
                for j in js:
                    sl = (b, u, pl.ds(n * 128, 128), pl.ds(j * 128, 128))
                    vbuf[sl] = vbuf[sl].T

        def softmax():
            s = s_scr[...].reshape(NG * G, W) * scale
            m = jnp.max(s, axis=-1, keepdims=True)
            p = jnp.exp(s - m)
            l = jnp.sum(p, axis=-1, keepdims=True)
            p_scr[...] = (p / l).reshape(NG, G, W)

        def attention_streaming(b, x):
            xn = _layernorm(x).astype(BF16)

            @pl.when(b == 0)
            def _():
                for c in wq_copies:
                    c.wait()

            def q_group(g, c):
                q_scr[g] = jnp.dot(xn, wq[g], preferred_element_type=F32)
                return c
            lax.fori_loop(0, NG, q_group, 0)

            k_copy(b, 0).wait()
            k_copy(b, 1).wait()

            def qk_group(g, c):
                qbd = jnp.where(diag, q_scr[g], 0.0).astype(BF16)
                for half in range(2):
                    s_scr[g, :, pl.ds(half * WH, WH)] = jnp.dot(
                        qbd, kbuf[b, half, pl.ds(pl.multiple_of(g * GD, GD), GD), :],
                        preferred_element_type=F32)
                return c
            lax.fori_loop(0, NG, qk_group, 0)
            softmax()

            def pv_wo(acc, pg, mask, v_rows, wo_rows):
                o = lax.dot_general(pg, v_rows, _NT, preferred_element_type=F32)
                o = jnp.where(mask, o, 0.0).astype(BF16)
                return acc + jnp.dot(o, wo_rows, preferred_element_type=F32)

            def group(g, acc):
                for r in range(2):
                    u = g * 2 + r

                    @pl.when(u > 0)
                    def _():
                        transpose_unit(b, u - 1)
                    if r == 0:
                        @pl.when(b < B - 1)
                        def _():
                            vgroup_copy(b, g).wait()

                    @pl.when(b == B - 1)
                    def _():
                        vunit_copy(u).wait()
                    acc = pv_wo(acc, p_scr[g].astype(BF16), diag_u[r], vbuf[b, u],
                                wo[pl.ds(pl.multiple_of(u * UD, UD), UD), :])
                return acc

            @pl.when(b == 0)
            def _():
                wo_copy.wait()
            acc = lax.fori_loop(0, NG - 1, group, jnp.zeros((8, D), F32))

            pg = p_scr[NG - 1].astype(BF16)
            transpose_unit(b, NU - 3)

            @pl.when(b < B - 1)
            def _():
                vgroup_copy(b, NG - 1).wait()

            @pl.when(b == B - 1)
            def _():
                vunit_copy(NU - 2).wait()
            acc = pv_wo(acc, pg, diag_u[0], vbuf[b, NU - 2], wo[pl.ds((NU - 2) * UD, UD), :])
            transpose_unit(b, NU - 2)
            for h, (r0, nr) in enumerate(LAST):
                @pl.when(b == B - 1)
                def _():
                    vlast_copy(h).wait()
                acc = pv_wo(acc, pg, diag_u[1][:, r0:r0 + nr], vbuf[b, NU - 1, pl.ds(r0, nr), :],
                            wo[pl.ds((NU - 1) * UD + r0, nr), :])
            return x + jnp.sum(acc, axis=0, keepdims=True)

        def attention_resident(b, x):
            xn = _layernorm(x).astype(BF16)
            KM = D - KV
            xcol[pl.ds(0, KV), :] = _columns(xn.astype(F32)[0:1, KM:])
            for g in range(NG):
                for n0 in (0, 6):
                    accs = [None] * 6
                    for kb in range(KV // 8):
                        cf = xcol[pl.ds(kb * 8, 8), :]
                        for t in range(6):
                            p = wq[g, pl.ds(KM + kb * 8, 8), pl.ds((n0 + t) * 128, 128)].astype(F32) * cf
                            accs[t] = p if accs[t] is None else accs[t] + p
                    for t in range(6):
                        n = n0 + t
                        q_scr[g, :, pl.ds(n * 128, 128)] = _bcast_sum(accs[t]) + jnp.dot(
                            xn[:, :KM], wq[g, pl.ds(0, KM), pl.ds(n * 128, 128)],
                            preferred_element_type=F32)
                transpose_unit(b, NU - 1, range(2 * g, 2 * g + 2))
            for g in range(NG):
                qbd = jnp.where(diag, q_scr[g], 0.0).astype(BF16)
                for half in range(2):
                    s_scr[g, :, pl.ds(half * WH, WH)] = jnp.dot(
                        qbd, kbuf[b, half, pl.ds(g * GD, GD), :], preferred_element_type=F32)
            softmax()
            outs = []
            for u in range(NU):
                pg = p_scr[u // 2].astype(BF16)
                tiles = []
                for n in range(UD // 128):
                    acc = None
                    for j in range(NJ):
                        d = jnp.dot(pg[:, j * 128:(j + 1) * 128],
                                    vbuf[b, u, pl.ds(n * 128, 128), pl.ds(j * 128, 128)],
                                    preferred_element_type=F32)
                        acc = d if acc is None else acc + d
                    tiles.append(acc)
                o = jnp.concatenate(tiles, axis=1)
                outs.append(jnp.where(diag_u[u % 2], o, 0.0).astype(BF16))
            acc = jnp.dot(jnp.concatenate(outs, axis=1), wo[...], preferred_element_type=F32)
            return x + jnp.sum(acc, axis=0, keepdims=True)

        def ffn(b, x, first):
            if first:
                @pl.when(b == 0)
                def _():
                    for c in ffn_copies:
                        c.wait()
            xnb = _layernorm(x).astype(BF16)
            xnr = xnb.astype(F32)
            r = jnp.sum(xnr * w_r, axis=-1, keepdims=True)
            xcol[...] = _columns(xnr[0:1, :])
            gu = []
            for w in (wg, wu):
                m = jnp.dot(xnb, w[:, pl.ds(0, (NTF - NV) * 128)], preferred_element_type=F32)
                accs = [None] * NV
                for kb in range(D // 8):
                    cf = xcol[pl.ds(kb * 8, 8), :]
                    for t in range(NV):
                        p = w[pl.ds(kb * 8, 8), pl.ds((NTF - NV + t) * 128, 128)].astype(F32) * cf
                        accs[t] = p if accs[t] is None else accs[t] + p
                gu.append(jnp.concatenate([m] + [_bcast_sum(a) for a in accs], axis=1))
            gate, up = gu
            h = (gate * jax.nn.sigmoid(gate) * up).astype(BF16)
            y = jnp.dot(h, wd[...], preferred_element_type=F32)
            return x + (xnr + y * jax.nn.sigmoid(r))

        def batch(b, carry):
            x = x_scr[b]
            x = attention_streaming(b, x)
            x = ffn(b, x, True)
            x = attention_resident(b, x)
            x = ffn(b, x, False)
            rows = lax.broadcasted_iota(jnp.int32, (8, D), 0)
            res = jnp.where(rows == b, x, res_scr[...])
            res_scr[...] = res
            o_scr[...] = res[0:B].astype(o_scr.dtype)
            return carry

        lax.fori_loop(0, B, batch, 0)

    def kernel(*refs):
        ins, out_ref, scratch, osem = refs[:9], refs[9], refs[10:-1], refs[-1]
        out_copy = pltpu.make_async_copy(scratch[-1], out_ref, osem)

        def scoped(sems):
            body(*ins, *scratch, sems)
            out_copy.start()
        pl.run_scoped(scoped, pltpu.SemaphoreType.DMA((NSEM,)))
        out_copy.wait()

    kt = jnp.transpose(A_k_cache, (0, 1, 3, 2)).reshape(B, HD, Sk)
    vt = jnp.transpose(A_v_cache, (0, 1, 3, 2)).reshape(B, NU, UD, Sk)
    x2 = A_x.reshape(B, D)

    hbm = pl.BlockSpec(memory_space=pltpu.HBM)
    out = pl.pallas_call(
        kernel,
        out_shape=jax.ShapeDtypeStruct((B, D), A_x.dtype),
        in_specs=[hbm] * 9,
        out_specs=hbm,
        scratch_shapes=[
            pltpu.VMEM((B, D), BF16),
            pltpu.VMEM((D,), BF16),
            pltpu.VMEM((B, 2, HD, WH), BF16),
            pltpu.VMEM((B, NU, UD, W), BF16),
            pltpu.VMEM((NG, D, GD), BF16),
            pltpu.VMEM((HD, D), BF16),
            pltpu.VMEM((D, F), BF16),
            pltpu.VMEM((D, F), BF16),
            pltpu.VMEM((F, D), BF16),
            pltpu.VMEM((B, 8, D), F32),
            pltpu.VMEM((NG, G, GD), F32),
            pltpu.VMEM((NG, G, W), F32),
            pltpu.VMEM((NG, G, W), F32),
            pltpu.VMEM((D, 128), F32),
            pltpu.VMEM((8, D), F32),
            pltpu.VMEM((B, D), BF16),
            pltpu.SemaphoreType.DMA(()),
        ],
        compiler_params=pltpu.CompilerParams(vmem_limit_bytes=127 * 1024 * 1024),
    )(x2, B_w_r, kt, vt, A_wq, A_wo, B_w_gate, B_w_up, B_w_down)
    return out.reshape(B, Sq, D)
```

```python
import jax
import jax.numpy as jnp
from jax import lax
import jax.experimental.pallas as pl
import jax.experimental.pallas.tpu as pltpu


F32 = jnp.float32
BF16 = jnp.bfloat16
_HQ, _DH = 32, 192
_NT = (((1,), (1,)), ((), ()))


def _layernorm(x, eps=1e-5):
    m = jnp.mean(x, axis=-1, keepdims=True)
    v = jnp.maximum(jnp.mean(x * x, axis=-1, keepdims=True) - m * m, 0.0)
    return (x - m) * lax.rsqrt(v + eps)


def _bcast_sum(a):
    return jnp.broadcast_to(jnp.sum(a, axis=0, keepdims=True), a.shape)


def _columns(rowvec):
    return jnp.broadcast_to(rowvec, (128, rowvec.shape[1])).T


@jax.jit
def pallas_interleave_layers__sliding_block_cached__moe_arch_mod__decode_kernel(
    A_x: jax.Array,
    A_k_cache: jax.Array,
    A_v_cache: jax.Array,
    A_wq: jax.Array,
    A_wo: jax.Array,
    B_x: jax.Array,
    B_w_r: jax.Array,
    B_w_gate: jax.Array,
    B_w_up: jax.Array,
    B_w_down: jax.Array,
):
    del B_x
    B, Sq, D = A_x.shape
    _, Hkv, Sk, Dh = A_k_cache.shape
    assert Sq == 1 and Hkv == _HQ and Dh == _DH
    F = B_w_gate.shape[1]
    W = min(4096, max(256, Sk // 4))
    HD = _HQ * _DH
    G = 8
    NG = _HQ // G
    GD = G * _DH
    NU = 2 * NG
    UD = HD // NU
    WH = W // 2
    NJ = W // 128
    NTF = F // 128
    LAST = ((0, 384), (384, 256), (640, 128))
    KV = 128
    NV = 2
    HO = 2
    scale = float(_DH) ** -0.5

    KS = 0
    VS = KS + B
    VL = VS + (B - 1) * NG
    WS = VL + NU - 1 + len(LAST)
    NSEM = WS + 4

    def body(x_hbm, wr_hbm, k_hbm, v_hbm, wq_hbm, wo_hbm, wg_hbm, wu_hbm, wd_hbm,
             xin, wr, kbuf, vbuf, wq, wo, wg, wu, wd,
             x_scr, q_scr, s_scr, p_scr, xcol, ocol, res_scr, o_scr, sems):

        def k_copy(b, half):
            return pltpu.make_async_copy(
                k_hbm.at[b, :, pl.ds(Sk - W + half * WH, WH)], kbuf.at[b, half], sems.at[KS + b])

        def vgroup_copy(b, g):
            return pltpu.make_async_copy(
                v_hbm.at[b, pl.ds(2 * g, 2), :, pl.ds(Sk - W, W)],
                vbuf.at[b, pl.ds(2 * g, 2)], sems.at[VS + b * NG + g])

        def vunit_copy(u):
            return pltpu.make_async_copy(
                v_hbm.at[B - 1, u, :, pl.ds(Sk - W, W)], vbuf.at[B - 1, u], sems.at[VL + u])

        def vlast_copy(h):
            r0, nr = LAST[h]
            return pltpu.make_async_copy(
                v_hbm.at[B - 1, NU - 1, pl.ds(r0, nr), pl.ds(Sk - W, W)],
                vbuf.at[B - 1, NU - 1, pl.ds(r0, nr)], sems.at[VL + NU - 1 + h])

        wq_copies = [pltpu.make_async_copy(wq_hbm.at[:, pl.ds(g * GD, GD)], wq.at[g], sems.at[WS])
                     for g in range(NG)]
        wo_copy = pltpu.make_async_copy(wo_hbm, wo, sems.at[WS + 1])
        ffn_copies = [pltpu.make_async_copy(s, d, sems.at[WS + 2])
                      for s, d in ((wg_hbm, wg), (wu_hbm, wu), (wd_hbm, wd))]
        row_copies = [pltpu.make_async_copy(x_hbm, xin, sems.at[WS + 3]),
                      pltpu.make_async_copy(wr_hbm, wr, sems.at[WS + 3])]

        for c in row_copies + wq_copies:
            c.start()
        k_copy(0, 0).start()
        k_copy(0, 1).start()
        wo_copy.start()
        for g in range(NG):
            vgroup_copy(0, g).start()
        for c in ffn_copies:
            c.start()
        for b in range(1, B):
            k_copy(b, 0).start()
            k_copy(b, 1).start()
            if b < B - 1:
                for g in range(NG):
                    vgroup_copy(b, g).start()
        for u in range(NU - 1):
            vunit_copy(u).start()
        for h in range(len(LAST)):
            vlast_copy(h).start()

        for c in row_copies:
            c.wait()
        x_in = xin[...].astype(F32)
        for b in range(B):
            x_scr[b] = jnp.broadcast_to(x_in[b:b + 1, :], (8, D))
        w_r = wr[...].astype(F32).reshape(1, D)
        res_scr[...] = jnp.zeros((8, D), F32)

        row = lax.broadcasted_iota(jnp.int32, (G, GD), 0)
        col = lax.broadcasted_iota(jnp.int32, (G, GD), 1)
        diag = (col >= row * _DH) & (col < (row + 1) * _DH)
        diag_u = [diag[:, :UD], diag[:, UD:]]

        def transpose_unit(b, u, js=range(NJ)):
            for n in range(UD // 128):
                for j in js:
                    sl = (b, u, pl.ds(n * 128, 128), pl.ds(j * 128, 128))
                    vbuf[sl] = vbuf[sl].T

        def softmax():
            s = s_scr[...].reshape(NG * G, W) * scale
            m = jnp.max(s, axis=-1, keepdims=True)
            p = jnp.exp(s - m)
            l = jnp.sum(p, axis=-1, keepdims=True)
            p_scr[...] = (p / l).reshape(NG, G, W)

        def attention_streaming(b, x):
            xn = _layernorm(x).astype(BF16)

            @pl.when(b == 0)
            def _():
                for c in wq_copies:
                    c.wait()

            def q_group(g, c):
                q_scr[g] = jnp.dot(xn, wq[g], preferred_element_type=F32)
                return c
            lax.fori_loop(0, NG, q_group, 0)

            k_copy(b, 0).wait()
            k_copy(b, 1).wait()

            def qk_group(g, c):
                qbd = jnp.where(diag, q_scr[g], 0.0).astype(BF16)
                for half in range(2):
                    s_scr[g, :, pl.ds(half * WH, WH)] = jnp.dot(
                        qbd, kbuf[b, half, pl.ds(pl.multiple_of(g * GD, GD), GD), :],
                        preferred_element_type=F32)
                return c
            lax.fori_loop(0, NG, qk_group, 0)
            softmax()

            def pv_wo(acc, pg, mask, v_rows, wo_rows):
                o = lax.dot_general(pg, v_rows, _NT, preferred_element_type=F32)
                o = jnp.where(mask, o, 0.0).astype(BF16)
                return acc + jnp.dot(o, wo_rows, preferred_element_type=F32)

            def group(g, acc):
                for r in range(2):
                    u = g * 2 + r

                    @pl.when(u > 0)
                    def _():
                        transpose_unit(b, u - 1)
                    if r == 0:
                        @pl.when(b < B - 1)
                        def _():
                            vgroup_copy(b, g).wait()

                    @pl.when(b == B - 1)
                    def _():
                        vunit_copy(u).wait()
                    acc = pv_wo(acc, p_scr[g].astype(BF16), diag_u[r], vbuf[b, u],
                                wo[pl.ds(pl.multiple_of(u * UD, UD), UD), :])
                return acc

            @pl.when(b == 0)
            def _():
                wo_copy.wait()
            acc = lax.fori_loop(0, NG - 1, group, jnp.zeros((8, D), F32))

            pg = p_scr[NG - 1].astype(BF16)
            transpose_unit(b, NU - 3)

            @pl.when(b < B - 1)
            def _():
                vgroup_copy(b, NG - 1).wait()

            @pl.when(b == B - 1)
            def _():
                vunit_copy(NU - 2).wait()
            acc = pv_wo(acc, pg, diag_u[0], vbuf[b, NU - 2], wo[pl.ds((NU - 2) * UD, UD), :])
            transpose_unit(b, NU - 2)
            for h, (r0, nr) in enumerate(LAST):
                @pl.when(b == B - 1)
                def _():
                    vlast_copy(h).wait()
                acc = pv_wo(acc, pg, diag_u[1][:, r0:r0 + nr], vbuf[b, NU - 1, pl.ds(r0, nr), :],
                            wo[pl.ds((NU - 1) * UD + r0, nr), :])
            return x + jnp.sum(acc, axis=0, keepdims=True)

        def attention_resident(b, x):
            xn = _layernorm(x).astype(BF16)
            KM = D - KV
            xcol[pl.ds(0, KV), :] = _columns(xn.astype(F32)[0:1, KM:])
            for g in range(NG):
                for n0 in (0, 6):
                    accs = [None] * 6
                    for kb in range(KV // 8):
                        cf = xcol[pl.ds(kb * 8, 8), :]
                        for t in range(6):
                            p = wq[g, pl.ds(KM + kb * 8, 8), pl.ds((n0 + t) * 128, 128)].astype(F32) * cf
                            accs[t] = p if accs[t] is None else accs[t] + p
                    for t in range(6):
                        n = n0 + t
                        q_scr[g, :, pl.ds(n * 128, 128)] = _bcast_sum(accs[t]) + jnp.dot(
                            xn[:, :KM], wq[g, pl.ds(0, KM), pl.ds(n * 128, 128)],
                            preferred_element_type=F32)
                transpose_unit(b, NU - 1, range(2 * g, 2 * g + 2))
            for g in range(NG):
                qbd = jnp.where(diag, q_scr[g], 0.0).astype(BF16)
                for half in range(2):
                    s_scr[g, :, pl.ds(half * WH, WH)] = jnp.dot(
                        qbd, kbuf[b, half, pl.ds(g * GD, GD), :], preferred_element_type=F32)
            softmax()
            outs = []
            for u in range(NU):
                pg = p_scr[u // 2].astype(BF16)
                tiles = []
                for n in range(UD // 128):
                    acc = None
                    for j in range(NJ):
                        d = jnp.dot(pg[:, j * 128:(j + 1) * 128],
                                    vbuf[b, u, pl.ds(n * 128, 128), pl.ds(j * 128, 128)],
                                    preferred_element_type=F32)
                        acc = d if acc is None else acc + d
                    tiles.append(acc)
                o = jnp.concatenate(tiles, axis=1)
                outs.append(jnp.where(diag_u[u % 2], o, 0.0).astype(BF16))
            acc = None
            for g in range(NG):
                og = jnp.concatenate(outs[2 * g:2 * g + 2], axis=1)
                MR = GD - (HO * _DH if g > 0 else 0)
                d = jnp.dot(og[:, :MR], wo[pl.ds(g * GD, MR), :], preferred_element_type=F32)
                if MR < GD:
                    ocol[g] = _columns(jnp.sum(og[:, MR:].astype(F32), axis=0, keepdims=True))
                    accs = [None] * (D // 128)
                    for rb in range((GD - MR) // 8):
                        cf = ocol[g, pl.ds(rb * 8, 8), :]
                        for t in range(D // 128):
                            p = wo[pl.ds(g * GD + MR + rb * 8, 8), pl.ds(t * 128, 128)].astype(F32) * cf
                            accs[t] = p if accs[t] is None else accs[t] + p
                    d = d + jnp.concatenate(accs, axis=1)
                acc = d if acc is None else acc + d
            return x + jnp.sum(acc, axis=0, keepdims=True)

        def ffn(b, x, first):
            if first:
                @pl.when(b == 0)
                def _():
                    for c in ffn_copies:
                        c.wait()
            xnb = _layernorm(x).astype(BF16)
            xnr = xnb.astype(F32)
            r = jnp.sum(xnr * w_r, axis=-1, keepdims=True)
            xcol[...] = _columns(xnr[0:1, :])
            gu = []
            for w in (wg, wu):
                m = jnp.dot(xnb, w[:, pl.ds(0, (NTF - NV) * 128)], preferred_element_type=F32)
                accs = [None] * NV
                for kb in range(D // 8):
                    cf = xcol[pl.ds(kb * 8, 8), :]
                    for t in range(NV):
                        p = w[pl.ds(kb * 8, 8), pl.ds((NTF - NV + t) * 128, 128)].astype(F32) * cf
                        accs[t] = p if accs[t] is None else accs[t] + p
                gu.append(jnp.concatenate([m] + [_bcast_sum(a) for a in accs], axis=1))
            gate, up = gu
            h = (gate * jax.nn.sigmoid(gate) * up).astype(BF16)
            y = jnp.dot(h, wd[...], preferred_element_type=F32)
            return x + (xnr + y * jax.nn.sigmoid(r))

        def batch(b, carry):
            x = x_scr[b]
            x = attention_streaming(b, x)
            x = ffn(b, x, True)
            x = attention_resident(b, x)
            x = ffn(b, x, False)
            rows = lax.broadcasted_iota(jnp.int32, (8, D), 0)
            res = jnp.where(rows == b, x, res_scr[...])
            res_scr[...] = res
            o_scr[...] = res[0:B].astype(o_scr.dtype)
            return carry

        lax.fori_loop(0, B, batch, 0)

    def kernel(*refs):
        ins, out_ref, scratch, osem = refs[:9], refs[9], refs[10:-1], refs[-1]
        out_copy = pltpu.make_async_copy(scratch[-1], out_ref, osem)

        def scoped(sems):
            body(*ins, *scratch, sems)
            out_copy.start()
        pl.run_scoped(scoped, pltpu.SemaphoreType.DMA((NSEM,)))
        out_copy.wait()

    kt = jnp.transpose(A_k_cache, (0, 1, 3, 2)).reshape(B, HD, Sk)
    vt = jnp.transpose(A_v_cache, (0, 1, 3, 2)).reshape(B, NU, UD, Sk)
    x2 = A_x.reshape(B, D)

    hbm = pl.BlockSpec(memory_space=pltpu.HBM)
    out = pl.pallas_call(
        kernel,
        out_shape=jax.ShapeDtypeStruct((B, D), A_x.dtype),
        in_specs=[hbm] * 9,
        out_specs=hbm,
        scratch_shapes=[
            pltpu.VMEM((B, D), BF16),
            pltpu.VMEM((D,), BF16),
            pltpu.VMEM((B, 2, HD, WH), BF16),
            pltpu.VMEM((B, NU, UD, W), BF16),
            pltpu.VMEM((NG, D, GD), BF16),
            pltpu.VMEM((HD, D), BF16),
            pltpu.VMEM((D, F), BF16),
            pltpu.VMEM((D, F), BF16),
            pltpu.VMEM((F, D), BF16),
            pltpu.VMEM((B, 8, D), F32),
            pltpu.VMEM((NG, G, GD), F32),
            pltpu.VMEM((NG, G, W), F32),
            pltpu.VMEM((NG, G, W), F32),
            pltpu.VMEM((D, 128), F32),
            pltpu.VMEM((NG, HO * _DH, 128), F32),
            pltpu.VMEM((8, D), F32),
            pltpu.VMEM((B, D), BF16),
            pltpu.SemaphoreType.DMA(()),
        ],
        compiler_params=pltpu.CompilerParams(vmem_limit_bytes=127 * 1024 * 1024),
    )(x2, B_w_r, kt, vt, A_wq, A_wo, B_w_gate, B_w_up, B_w_down)
    return out.reshape(B, Sq, D)
```

```python
import jax
import jax.numpy as jnp
from jax import lax
import jax.experimental.pallas as pl
import jax.experimental.pallas.tpu as pltpu


F32 = jnp.float32
BF16 = jnp.bfloat16
_HQ, _DH = 32, 192
_NT = (((1,), (1,)), ((), ()))


def _layernorm(x, eps=1e-5):
    m = jnp.mean(x, axis=-1, keepdims=True)
    v = jnp.maximum(jnp.mean(x * x, axis=-1, keepdims=True) - m * m, 0.0)
    return (x - m) * lax.rsqrt(v + eps)


def _ln_split(x, eps=1e-5):
    xb = x.astype(BF16)
    xr = xb.astype(F32)
    m = jnp.mean(xr, axis=-1, keepdims=True)
    v = jnp.maximum(jnp.mean(xr * xr, axis=-1, keepdims=True) - m * m, 0.0)
    rstd = lax.rsqrt(v + eps)
    lhs = jnp.concatenate([xb, jnp.ones_like(xb)], axis=0)
    return lhs, m, rstd, ((xr - m) * rstd).astype(BF16)


def _bcast_sum(a):
    return jnp.broadcast_to(jnp.sum(a, axis=0, keepdims=True), a.shape)


def _columns(rowvec):
    return jnp.broadcast_to(rowvec, (128, rowvec.shape[1])).T


@jax.jit
def pallas_interleave_layers__sliding_block_cached__moe_arch_mod__decode_kernel(
    A_x: jax.Array,
    A_k_cache: jax.Array,
    A_v_cache: jax.Array,
    A_wq: jax.Array,
    A_wo: jax.Array,
    B_x: jax.Array,
    B_w_r: jax.Array,
    B_w_gate: jax.Array,
    B_w_up: jax.Array,
    B_w_down: jax.Array,
):
    del B_x
    B, Sq, D = A_x.shape
    _, Hkv, Sk, Dh = A_k_cache.shape
    assert Sq == 1 and Hkv == _HQ and Dh == _DH
    F = B_w_gate.shape[1]
    W = min(4096, max(256, Sk // 4))
    HD = _HQ * _DH
    G = 8
    NG = _HQ // G
    GD = G * _DH
    NU = 2 * NG
    UD = HD // NU
    WH = W // 2
    NJ = W // 128
    NTF = F // 128
    LAST = ((0, 384), (384, 256), (640, 128))
    KV = 128
    NV = 2
    HO = 2
    scale = float(_DH) ** -0.5

    KS = 0
    VS = KS + B
    VL = VS + (B - 1) * NG
    WS = VL + NU - 1 + len(LAST)
    NSEM = WS + 4

    def body(x_hbm, wr_hbm, k_hbm, v_hbm, wq_hbm, wo_hbm, wg_hbm, wu_hbm, wd_hbm,
             xin, wr, kbuf, vbuf, wq, wo, wg, wu, wd,
             x_scr, q_scr, s_scr, p_scr, xcol, ocol, res_scr, o_scr, sems):

        def k_copy(b, half):
            return pltpu.make_async_copy(
                k_hbm.at[b, :, pl.ds(Sk - W + half * WH, WH)], kbuf.at[b, half], sems.at[KS + b])

        def vgroup_copy(b, g):
            return pltpu.make_async_copy(
                v_hbm.at[b, pl.ds(2 * g, 2), :, pl.ds(Sk - W, W)],
                vbuf.at[b, pl.ds(2 * g, 2)], sems.at[VS + b * NG + g])

        def vunit_copy(u):
            return pltpu.make_async_copy(
                v_hbm.at[B - 1, u, :, pl.ds(Sk - W, W)], vbuf.at[B - 1, u], sems.at[VL + u])

        def vlast_copy(h):
            r0, nr = LAST[h]
            return pltpu.make_async_copy(
                v_hbm.at[B - 1, NU - 1, pl.ds(r0, nr), pl.ds(Sk - W, W)],
                vbuf.at[B - 1, NU - 1, pl.ds(r0, nr)], sems.at[VL + NU - 1 + h])

        wq_copies = [pltpu.make_async_copy(wq_hbm.at[:, pl.ds(g * GD, GD)], wq.at[g], sems.at[WS])
                     for g in range(NG)]
        wo_copy = pltpu.make_async_copy(wo_hbm, wo, sems.at[WS + 1])
        ffn_copies = [pltpu.make_async_copy(s, d, sems.at[WS + 2])
                      for s, d in ((wg_hbm, wg), (wu_hbm, wu), (wd_hbm, wd))]
        row_copies = [pltpu.make_async_copy(x_hbm, xin, sems.at[WS + 3]),
                      pltpu.make_async_copy(wr_hbm, wr, sems.at[WS + 3])]

        for c in row_copies + wq_copies:
            c.start()
        k_copy(0, 0).start()
        k_copy(0, 1).start()
        wo_copy.start()
        for g in range(NG):
            vgroup_copy(0, g).start()
        for c in ffn_copies:
            c.start()
        for b in range(1, B):
            k_copy(b, 0).start()
            k_copy(b, 1).start()
            if b < B - 1:
                for g in range(NG):
                    vgroup_copy(b, g).start()
        for u in range(NU - 1):
            vunit_copy(u).start()
        for h in range(len(LAST)):
            vlast_copy(h).start()

        for c in row_copies:
            c.wait()
        x_in = xin[...].astype(F32)
        for b in range(B):
            x_scr[b] = jnp.broadcast_to(x_in[b:b + 1, :], (8, D))
        w_r = wr[...].astype(F32).reshape(1, D)
        res_scr[...] = jnp.zeros((8, D), F32)

        row = lax.broadcasted_iota(jnp.int32, (G, GD), 0)
        col = lax.broadcasted_iota(jnp.int32, (G, GD), 1)
        diag = (col >= row * _DH) & (col < (row + 1) * _DH)
        diag_u = [diag[:, :UD], diag[:, UD:]]

        def transpose_unit(b, u, js=range(NJ)):
            for n in range(UD // 128):
                for j in js:
                    sl = (b, u, pl.ds(n * 128, 128), pl.ds(j * 128, 128))
                    vbuf[sl] = vbuf[sl].T

        def softmax():
            s = s_scr[...].reshape(NG * G, W) * scale
            m = jnp.max(s, axis=-1, keepdims=True)
            p = jnp.exp(s - m)
            l = jnp.sum(p, axis=-1, keepdims=True)
            p_scr[...] = (p / l).reshape(NG, G, W)

        def attention_streaming(b, x):
            xn = _layernorm(x).astype(BF16)

            @pl.when(b == 0)
            def _():
                for c in wq_copies:
                    c.wait()

            def q_group(g, c):
                q_scr[g] = jnp.dot(xn, wq[g], preferred_element_type=F32)
                return c
            lax.fori_loop(0, NG, q_group, 0)

            k_copy(b, 0).wait()
            k_copy(b, 1).wait()

            def qk_group(g, c):
                qbd = jnp.where(diag, q_scr[g], 0.0).astype(BF16)
                for half in range(2):
                    s_scr[g, :, pl.ds(half * WH, WH)] = jnp.dot(
                        qbd, kbuf[b, half, pl.ds(pl.multiple_of(g * GD, GD), GD), :],
                        preferred_element_type=F32)
                return c
            lax.fori_loop(0, NG, qk_group, 0)
            softmax()

            def pv_wo(acc, pg, mask, v_rows, wo_rows):
                o = lax.dot_general(pg, v_rows, _NT, preferred_element_type=F32)
                o = jnp.where(mask, o, 0.0).astype(BF16)
                return acc + jnp.dot(o, wo_rows, preferred_element_type=F32)

            def group(g, acc):
                for r in range(2):
                    u = g * 2 + r

                    @pl.when(u > 0)
                    def _():
                        transpose_unit(b, u - 1)
                    if r == 0:
                        @pl.when(b < B - 1)
                        def _():
                            vgroup_copy(b, g).wait()

                    @pl.when(b == B - 1)
                    def _():
                        vunit_copy(u).wait()
                    acc = pv_wo(acc, p_scr[g].astype(BF16), diag_u[r], vbuf[b, u],
                                wo[pl.ds(pl.multiple_of(u * UD, UD), UD), :])
                return acc

            @pl.when(b == 0)
            def _():
                wo_copy.wait()
            acc = lax.fori_loop(0, NG - 1, group, jnp.zeros((8, D), F32))

            pg = p_scr[NG - 1].astype(BF16)
            transpose_unit(b, NU - 3)

            @pl.when(b < B - 1)
            def _():
                vgroup_copy(b, NG - 1).wait()

            @pl.when(b == B - 1)
            def _():
                vunit_copy(NU - 2).wait()
            acc = pv_wo(acc, pg, diag_u[0], vbuf[b, NU - 2], wo[pl.ds((NU - 2) * UD, UD), :])
            transpose_unit(b, NU - 2)
            for h, (r0, nr) in enumerate(LAST):
                @pl.when(b == B - 1)
                def _():
                    vlast_copy(h).wait()
                acc = pv_wo(acc, pg, diag_u[1][:, r0:r0 + nr], vbuf[b, NU - 1, pl.ds(r0, nr), :],
                            wo[pl.ds((NU - 1) * UD + r0, nr), :])
            return x + jnp.sum(acc, axis=0, keepdims=True)

        def attention_resident(b, x):
            lhs, mu, rstd, xn = _ln_split(x)
            KM = D - KV
            xcol[pl.ds(0, KV), :] = _columns(xn.astype(F32)[0:1, KM:])
            for g in range(NG):
                for n0 in (0, 6):
                    accs = [None] * 6
                    for kb in range(KV // 8):
                        cf = xcol[pl.ds(kb * 8, 8), :]
                        for t in range(6):
                            p = wq[g, pl.ds(KM + kb * 8, 8), pl.ds((n0 + t) * 128, 128)].astype(F32) * cf
                            accs[t] = p if accs[t] is None else accs[t] + p
                    for t in range(6):
                        n = n0 + t
                        d = jnp.dot(lhs[:, :KM], wq[g, pl.ds(0, KM), pl.ds(n * 128, 128)],
                                    preferred_element_type=F32)
                        q_scr[g, :, pl.ds(n * 128, 128)] = (
                            _bcast_sum(accs[t]) + (d[0:8] - mu * d[8:16]) * rstd)
                transpose_unit(b, NU - 1, range(2 * g, 2 * g + 2))
            for g in range(NG):
                qbd = jnp.where(diag, q_scr[g], 0.0).astype(BF16)
                for half in range(2):
                    s_scr[g, :, pl.ds(half * WH, WH)] = jnp.dot(
                        qbd, kbuf[b, half, pl.ds(g * GD, GD), :], preferred_element_type=F32)
            softmax()
            outs = []
            for u in range(NU):
                pg = p_scr[u // 2].astype(BF16)
                tiles = []
                for n in range(UD // 128):
                    acc = None
                    for j in range(NJ):
                        d = jnp.dot(pg[:, j * 128:(j + 1) * 128],
                                    vbuf[b, u, pl.ds(n * 128, 128), pl.ds(j * 128, 128)],
                                    preferred_element_type=F32)
                        acc = d if acc is None else acc + d
                    tiles.append(acc)
                o = jnp.concatenate(tiles, axis=1)
                outs.append(jnp.where(diag_u[u % 2], o, 0.0).astype(BF16))
            acc = None
            for g in range(NG):
                og = jnp.concatenate(outs[2 * g:2 * g + 2], axis=1)
                MR = GD - (HO * _DH if g > 0 else 0)
                d = jnp.dot(og[:, :MR], wo[pl.ds(g * GD, MR), :], preferred_element_type=F32)
                if MR < GD:
                    ocol[g] = _columns(jnp.sum(og[:, MR:].astype(F32), axis=0, keepdims=True))
                    accs = [None] * (D // 128)
                    for rb in range((GD - MR) // 8):
                        cf = ocol[g, pl.ds(rb * 8, 8), :]
                        for t in range(D // 128):
                            p = wo[pl.ds(g * GD + MR + rb * 8, 8), pl.ds(t * 128, 128)].astype(F32) * cf
                            accs[t] = p if accs[t] is None else accs[t] + p
                    d = d + jnp.concatenate(accs, axis=1)
                acc = d if acc is None else acc + d
            return x + jnp.sum(acc, axis=0, keepdims=True)

        def ffn(b, x, first):
            if first:
                @pl.when(b == 0)
                def _():
                    for c in ffn_copies:
                        c.wait()
            lhs, mu, rstd, xnb = _ln_split(x)
            xnr = xnb.astype(F32)
            r = jnp.sum(xnr * w_r, axis=-1, keepdims=True)
            xcol[...] = _columns(xnr[0:1, :])
            gu = []
            for w in (wg, wu):
                m = jnp.dot(lhs, w[:, pl.ds(0, (NTF - NV) * 128)], preferred_element_type=F32)
                m = (m[0:8] - mu * m[8:16]) * rstd
                accs = [None] * NV
                for kb in range(D // 8):
                    cf = xcol[pl.ds(kb * 8, 8), :]
                    for t in range(NV):
                        p = w[pl.ds(kb * 8, 8), pl.ds((NTF - NV + t) * 128, 128)].astype(F32) * cf
                        accs[t] = p if accs[t] is None else accs[t] + p
                gu.append(jnp.concatenate([m] + [_bcast_sum(a) for a in accs], axis=1))
            gate, up = gu
            h = (gate * jax.nn.sigmoid(gate) * up).astype(BF16)
            y = jnp.dot(h, wd[...], preferred_element_type=F32)
            return x + (xnr + y * jax.nn.sigmoid(r))

        def batch(b, carry):
            x = x_scr[b]
            x = attention_streaming(b, x)
            x = ffn(b, x, True)
            x = attention_resident(b, x)
            x = ffn(b, x, False)
            rows = lax.broadcasted_iota(jnp.int32, (8, D), 0)
            res = jnp.where(rows == b, x, res_scr[...])
            res_scr[...] = res
            o_scr[...] = res[0:B].astype(o_scr.dtype)
            return carry

        lax.fori_loop(0, B, batch, 0)

    def kernel(*refs):
        ins, out_ref, scratch, osem = refs[:9], refs[9], refs[10:-1], refs[-1]
        out_copy = pltpu.make_async_copy(scratch[-1], out_ref, osem)

        def scoped(sems):
            body(*ins, *scratch, sems)
            out_copy.start()
        pl.run_scoped(scoped, pltpu.SemaphoreType.DMA((NSEM,)))
        out_copy.wait()

    kt = jnp.transpose(A_k_cache, (0, 1, 3, 2)).reshape(B, HD, Sk)
    vt = jnp.transpose(A_v_cache, (0, 1, 3, 2)).reshape(B, NU, UD, Sk)
    x2 = A_x.reshape(B, D)

    hbm = pl.BlockSpec(memory_space=pltpu.HBM)
    out = pl.pallas_call(
        kernel,
        out_shape=jax.ShapeDtypeStruct((B, D), A_x.dtype),
        in_specs=[hbm] * 9,
        out_specs=hbm,
        scratch_shapes=[
            pltpu.VMEM((B, D), BF16),
            pltpu.VMEM((D,), BF16),
            pltpu.VMEM((B, 2, HD, WH), BF16),
            pltpu.VMEM((B, NU, UD, W), BF16),
            pltpu.VMEM((NG, D, GD), BF16),
            pltpu.VMEM((HD, D), BF16),
            pltpu.VMEM((D, F), BF16),
            pltpu.VMEM((D, F), BF16),
            pltpu.VMEM((F, D), BF16),
            pltpu.VMEM((B, 8, D), F32),
            pltpu.VMEM((NG, G, GD), F32),
            pltpu.VMEM((NG, G, W), F32),
            pltpu.VMEM((NG, G, W), F32),
            pltpu.VMEM((D, 128), F32),
            pltpu.VMEM((NG, HO * _DH, 128), F32),
            pltpu.VMEM((8, D), F32),
            pltpu.VMEM((B, D), BF16),
            pltpu.SemaphoreType.DMA(()),
        ],
        compiler_params=pltpu.CompilerParams(vmem_limit_bytes=127 * 1024 * 1024),
    )(x2, B_w_r, kt, vt, A_wq, A_wo, B_w_gate, B_w_up, B_w_down)
    return out.reshape(B, Sq, D)
```

```python
import jax
import jax.numpy as jnp
from jax import lax
import jax.experimental.pallas as pl
import jax.experimental.pallas.tpu as pltpu


F32 = jnp.float32
BF16 = jnp.bfloat16
_HQ, _DH = 32, 192
_NT = (((1,), (1,)), ((), ()))


def _layernorm(x, eps=1e-5):
    m = jnp.mean(x, axis=-1, keepdims=True)
    xc = x - m
    v = jnp.mean(xc * xc, axis=-1, keepdims=True)
    return xc * lax.rsqrt(v + eps)


def _ln_split(x, eps=1e-5):
    xb = x.astype(BF16)
    xr = xb.astype(F32)
    m = jnp.mean(xr, axis=-1, keepdims=True)
    xc = xr - m
    v = jnp.mean(xc * xc, axis=-1, keepdims=True)
    rstd = lax.rsqrt(v + eps)
    lhs = jnp.concatenate([xb, jnp.ones_like(xb)], axis=0)
    return lhs, m, rstd, (xc * rstd).astype(BF16)


def _bcast_sum(a):
    return jnp.broadcast_to(jnp.sum(a, axis=0, keepdims=True), a.shape)


def _columns(rowvec):
    return jnp.broadcast_to(rowvec, (128, rowvec.shape[1])).T


@jax.jit
def pallas_interleave_layers__sliding_block_cached__moe_arch_mod__decode_kernel(
    A_x: jax.Array,
    A_k_cache: jax.Array,
    A_v_cache: jax.Array,
    A_wq: jax.Array,
    A_wo: jax.Array,
    B_x: jax.Array,
    B_w_r: jax.Array,
    B_w_gate: jax.Array,
    B_w_up: jax.Array,
    B_w_down: jax.Array,
):
    del B_x
    B, Sq, D = A_x.shape
    _, Hkv, Sk, Dh = A_k_cache.shape
    assert Sq == 1 and Hkv == _HQ and Dh == _DH
    F = B_w_gate.shape[1]
    W = min(4096, max(256, Sk // 4))
    HD = _HQ * _DH
    G = 8
    NG = _HQ // G
    GD = G * _DH
    NU = 2 * NG
    UD = HD // NU
    WH = W // 2
    NJ = W // 128
    NTF = F // 128
    LAST = ((0, 384), (384, 256), (640, 128))
    KV = 128
    NV = 2
    HO = 2
    scale = float(_DH) ** -0.5

    KS = 0
    VS = KS + B
    VL = VS + (B - 1) * NG
    WS = VL + NU - 1 + len(LAST)
    NSEM = WS + 4

    def body(x_hbm, wr_hbm, k_hbm, v_hbm, wq_hbm, wo_hbm, wg_hbm, wu_hbm, wd_hbm,
             xin, wr, kbuf, vbuf, wq, wo, wg, wu, wd,
             x_scr, q_scr, s_scr, p_scr, xcol, ocol, res_scr, o_scr, sems):

        def k_copy(b, half):
            return pltpu.make_async_copy(
                k_hbm.at[b, :, pl.ds(Sk - W + half * WH, WH)], kbuf.at[b, half], sems.at[KS + b])

        def vgroup_copy(b, g):
            return pltpu.make_async_copy(
                v_hbm.at[b, pl.ds(2 * g, 2), :, pl.ds(Sk - W, W)],
                vbuf.at[b, pl.ds(2 * g, 2)], sems.at[VS + b * NG + g])

        def vunit_copy(u):
            return pltpu.make_async_copy(
                v_hbm.at[B - 1, u, :, pl.ds(Sk - W, W)], vbuf.at[B - 1, u], sems.at[VL + u])

        def vlast_copy(h):
            r0, nr = LAST[h]
            return pltpu.make_async_copy(
                v_hbm.at[B - 1, NU - 1, pl.ds(r0, nr), pl.ds(Sk - W, W)],
                vbuf.at[B - 1, NU - 1, pl.ds(r0, nr)], sems.at[VL + NU - 1 + h])

        wq_copies = [pltpu.make_async_copy(wq_hbm.at[:, pl.ds(g * GD, GD)], wq.at[g], sems.at[WS])
                     for g in range(NG)]
        wo_copy = pltpu.make_async_copy(wo_hbm, wo, sems.at[WS + 1])
        ffn_copies = [pltpu.make_async_copy(s, d, sems.at[WS + 2])
                      for s, d in ((wg_hbm, wg), (wu_hbm, wu), (wd_hbm, wd))]
        row_copies = [pltpu.make_async_copy(x_hbm, xin, sems.at[WS + 3]),
                      pltpu.make_async_copy(wr_hbm, wr, sems.at[WS + 3])]

        for c in row_copies + wq_copies:
            c.start()
        k_copy(0, 0).start()
        k_copy(0, 1).start()
        wo_copy.start()
        for g in range(NG):
            vgroup_copy(0, g).start()
        for c in ffn_copies:
            c.start()
        for b in range(1, B):
            k_copy(b, 0).start()
            k_copy(b, 1).start()
            if b < B - 1:
                for g in range(NG):
                    vgroup_copy(b, g).start()
        for u in range(NU - 1):
            vunit_copy(u).start()
        for h in range(len(LAST)):
            vlast_copy(h).start()

        for c in row_copies:
            c.wait()
        x_in = xin[...].astype(F32)
        for b in range(B):
            x_scr[b] = jnp.broadcast_to(x_in[b:b + 1, :], (8, D))
        w_r = wr[...].astype(F32).reshape(1, D)
        res_scr[...] = jnp.zeros((8, D), F32)

        row = lax.broadcasted_iota(jnp.int32, (G, GD), 0)
        col = lax.broadcasted_iota(jnp.int32, (G, GD), 1)
        diag = (col >= row * _DH) & (col < (row + 1) * _DH)
        diag_u = [diag[:, :UD], diag[:, UD:]]

        def transpose_unit(b, u, js=range(NJ)):
            for n in range(UD // 128):
                for j in js:
                    sl = (b, u, pl.ds(n * 128, 128), pl.ds(j * 128, 128))
                    vbuf[sl] = vbuf[sl].T

        def softmax():
            s = s_scr[...].reshape(NG * G, W) * scale
            m = jnp.max(s, axis=-1, keepdims=True)
            p = jnp.exp(s - m)
            l = jnp.sum(p, axis=-1, keepdims=True)
            p_scr[...] = (p / l).reshape(NG, G, W)

        def attention_streaming(b, x):
            xn = _layernorm(x).astype(BF16)

            @pl.when(b == 0)
            def _():
                for c in wq_copies:
                    c.wait()

            def q_group(g, c):
                q_scr[g] = jnp.dot(xn, wq[g], preferred_element_type=F32)
                return c
            lax.fori_loop(0, NG, q_group, 0)

            k_copy(b, 0).wait()
            k_copy(b, 1).wait()

            def qk_group(g, c):
                qbd = jnp.where(diag, q_scr[g], 0.0).astype(BF16)
                for half in range(2):
                    s_scr[g, :, pl.ds(half * WH, WH)] = jnp.dot(
                        qbd, kbuf[b, half, pl.ds(pl.multiple_of(g * GD, GD), GD), :],
                        preferred_element_type=F32)
                return c
            lax.fori_loop(0, NG, qk_group, 0)
            softmax()

            def pv_wo(acc, pg, mask, v_rows, wo_rows):
                o = lax.dot_general(pg, v_rows, _NT, preferred_element_type=F32)
                o = jnp.where(mask, o, 0.0).astype(BF16)
                return acc + jnp.dot(o, wo_rows, preferred_element_type=F32)

            def group(g, acc):
                for r in range(2):
                    u = g * 2 + r

                    @pl.when(u > 0)
                    def _():
                        transpose_unit(b, u - 1)
                    if r == 0:
                        @pl.when(b < B - 1)
                        def _():
                            vgroup_copy(b, g).wait()

                    @pl.when(b == B - 1)
                    def _():
                        vunit_copy(u).wait()
                    acc = pv_wo(acc, p_scr[g].astype(BF16), diag_u[r], vbuf[b, u],
                                wo[pl.ds(pl.multiple_of(u * UD, UD), UD), :])
                return acc

            @pl.when(b == 0)
            def _():
                wo_copy.wait()
            acc = lax.fori_loop(0, NG - 1, group, jnp.zeros((8, D), F32))

            pg = p_scr[NG - 1].astype(BF16)
            transpose_unit(b, NU - 3)

            @pl.when(b < B - 1)
            def _():
                vgroup_copy(b, NG - 1).wait()

            @pl.when(b == B - 1)
            def _():
                vunit_copy(NU - 2).wait()
            acc = pv_wo(acc, pg, diag_u[0], vbuf[b, NU - 2], wo[pl.ds((NU - 2) * UD, UD), :])
            transpose_unit(b, NU - 2)
            for h, (r0, nr) in enumerate(LAST):
                @pl.when(b == B - 1)
                def _():
                    vlast_copy(h).wait()
                acc = pv_wo(acc, pg, diag_u[1][:, r0:r0 + nr], vbuf[b, NU - 1, pl.ds(r0, nr), :],
                            wo[pl.ds((NU - 1) * UD + r0, nr), :])
            return x + jnp.sum(acc, axis=0, keepdims=True)

        def attention_resident(b, x):
            lhs, mu, rstd, xn = _ln_split(x)
            KM = D - KV
            xcol[pl.ds(0, KV), :] = _columns(xn.astype(F32)[0:1, KM:])
            for g in range(NG):
                for n0 in (0, 6):
                    accs = [None] * 6
                    for kb in range(KV // 8):
                        cf = xcol[pl.ds(kb * 8, 8), :]
                        for t in range(6):
                            p = wq[g, pl.ds(KM + kb * 8, 8), pl.ds((n0 + t) * 128, 128)].astype(F32) * cf
                            accs[t] = p if accs[t] is None else accs[t] + p
                    for t in range(6):
                        n = n0 + t
                        d = jnp.dot(lhs[:, :KM], wq[g, pl.ds(0, KM), pl.ds(n * 128, 128)],
                                    preferred_element_type=F32)
                        q_scr[g, :, pl.ds(n * 128, 128)] = (
                            _bcast_sum(accs[t]) + (d[0:8] - mu * d[8:16]) * rstd)
                transpose_unit(b, NU - 1, range(2 * g, 2 * g + 2))
            for g in range(NG):
                qbd = jnp.where(diag, q_scr[g], 0.0).astype(BF16)
                for half in range(2):
                    s_scr[g, :, pl.ds(half * WH, WH)] = jnp.dot(
                        qbd, kbuf[b, half, pl.ds(g * GD, GD), :], preferred_element_type=F32)
            softmax()
            outs = []
            for u in range(NU):
                pg = p_scr[u // 2].astype(BF16)
                tiles = []
                for n in range(UD // 128):
                    acc = None
                    for j in range(NJ):
                        d = jnp.dot(pg[:, j * 128:(j + 1) * 128],
                                    vbuf[b, u, pl.ds(n * 128, 128), pl.ds(j * 128, 128)],
                                    preferred_element_type=F32)
                        acc = d if acc is None else acc + d
                    tiles.append(acc)
                o = jnp.concatenate(tiles, axis=1)
                outs.append(jnp.where(diag_u[u % 2], o, 0.0).astype(BF16))
            acc = None
            for g in range(NG):
                og = jnp.concatenate(outs[2 * g:2 * g + 2], axis=1)
                MR = GD - (HO * _DH if g > 0 else 0)
                d = jnp.dot(og[:, :MR], wo[pl.ds(g * GD, MR), :], preferred_element_type=F32)
                if MR < GD:
                    ocol[g] = _columns(jnp.sum(og[:, MR:].astype(F32), axis=0, keepdims=True))
                    accs = [None] * (D // 128)
                    for rb in range((GD - MR) // 8):
                        cf = ocol[g, pl.ds(rb * 8, 8), :]
                        for t in range(D // 128):
                            p = wo[pl.ds(g * GD + MR + rb * 8, 8), pl.ds(t * 128, 128)].astype(F32) * cf
                            accs[t] = p if accs[t] is None else accs[t] + p
                    d = d + jnp.concatenate(accs, axis=1)
                acc = d if acc is None else acc + d
            return x + jnp.sum(acc, axis=0, keepdims=True)

        def ffn(b, x, first):
            if first:
                @pl.when(b == 0)
                def _():
                    for c in ffn_copies:
                        c.wait()
            lhs, mu, rstd, xnb = _ln_split(x)
            xnr = xnb.astype(F32)
            r = jnp.sum(xnr * w_r, axis=-1, keepdims=True)
            xcol[...] = _columns(xnr[0:1, :])
            gu = []
            for w in (wg, wu):
                m = jnp.dot(lhs, w[:, pl.ds(0, (NTF - NV) * 128)], preferred_element_type=F32)
                m = (m[0:8] - mu * m[8:16]) * rstd
                accs = [None] * NV
                for kb in range(D // 8):
                    cf = xcol[pl.ds(kb * 8, 8), :]
                    for t in range(NV):
                        p = w[pl.ds(kb * 8, 8), pl.ds((NTF - NV + t) * 128, 128)].astype(F32) * cf
                        accs[t] = p if accs[t] is None else accs[t] + p
                gu.append(jnp.concatenate([m] + [_bcast_sum(a) for a in accs], axis=1))
            gate, up = gu
            h = (gate * jax.nn.sigmoid(gate) * up).astype(BF16)
            y = jnp.dot(h, wd[...], preferred_element_type=F32)
            return x + (xnr + y * jax.nn.sigmoid(r))

        def batch(b, carry):
            x = x_scr[b]
            x = attention_streaming(b, x)
            x = ffn(b, x, True)
            x = attention_resident(b, x)
            x = ffn(b, x, False)
            rows = lax.broadcasted_iota(jnp.int32, (8, D), 0)
            res = jnp.where(rows == b, x, res_scr[...])
            res_scr[...] = res
            o_scr[...] = res[0:B].astype(o_scr.dtype)
            return carry

        lax.fori_loop(0, B, batch, 0)

    def kernel(*refs):
        ins, out_ref, scratch, osem = refs[:9], refs[9], refs[10:-1], refs[-1]
        out_copy = pltpu.make_async_copy(scratch[-1], out_ref, osem)

        def scoped(sems):
            body(*ins, *scratch, sems)
            out_copy.start()
        pl.run_scoped(scoped, pltpu.SemaphoreType.DMA((NSEM,)))
        out_copy.wait()

    kt = jnp.transpose(A_k_cache, (0, 1, 3, 2)).reshape(B, HD, Sk)
    vt = jnp.transpose(A_v_cache, (0, 1, 3, 2)).reshape(B, NU, UD, Sk)
    x2 = A_x.reshape(B, D)

    hbm = pl.BlockSpec(memory_space=pltpu.HBM)
    out = pl.pallas_call(
        kernel,
        out_shape=jax.ShapeDtypeStruct((B, D), A_x.dtype),
        in_specs=[hbm] * 9,
        out_specs=hbm,
        scratch_shapes=[
            pltpu.VMEM((B, D), BF16),
            pltpu.VMEM((D,), BF16),
            pltpu.VMEM((B, 2, HD, WH), BF16),
            pltpu.VMEM((B, NU, UD, W), BF16),
            pltpu.VMEM((NG, D, GD), BF16),
            pltpu.VMEM((HD, D), BF16),
            pltpu.VMEM((D, F), BF16),
            pltpu.VMEM((D, F), BF16),
            pltpu.VMEM((F, D), BF16),
            pltpu.VMEM((B, 8, D), F32),
            pltpu.VMEM((NG, G, GD), F32),
            pltpu.VMEM((NG, G, W), F32),
            pltpu.VMEM((NG, G, W), F32),
            pltpu.VMEM((D, 128), F32),
            pltpu.VMEM((NG, HO * _DH, 128), F32),
            pltpu.VMEM((8, D), F32),
            pltpu.VMEM((B, D), BF16),
            pltpu.SemaphoreType.DMA(()),
        ],
        compiler_params=pltpu.CompilerParams(vmem_limit_bytes=127 * 1024 * 1024),
    )(x2, B_w_r, kt, vt, A_wq, A_wo, B_w_gate, B_w_up, B_w_down)
    return out.reshape(B, Sq, D)
```
